```python
import jax
import jax.numpy as jnp

def _softmax(x, axis=-1):
    return jax.nn.softmax(x, axis=axis)

def _gelu(x):
    return jax.nn.gelu(x, approximate=True)

def _silu(x):
    return jax.nn.silu(x)

def _sigmoid(x):
    return jax.nn.sigmoid(x)

def _layernorm(x, axis=-1, eps=1e-05):
    m = jnp.mean(x, axis=axis, keepdims=True)
    v = jnp.var(x, axis=axis, keepdims=True)
    return (x - m) / jnp.sqrt(v + eps)

def _scatter_add(tgt, idx, src, axis=0):
    return tgt.at[idx].add(src)

def _segment_sum(src, seg, n):
    return jax.ops.segment_sum(src, seg, n)

class _Rng:

    def __init__(self, key):
        self._k = key

    def _next(self):
        self._k, sub = jax.random.split(self._k)
        return sub

    def normal(self, shape):
        return jax.random.normal(self._next(), shape, dtype=jnp.bfloat16)

    def randint(self, lo, hi, shape):
        return jax.random.randint(self._next(), shape, lo, hi, dtype=jnp.int32)

    def uniform(self, shape, lo=0.0, hi=1.0):
        return jax.random.uniform(self._next(), shape, jnp.bfloat16, lo, hi)

    def permutation(self, n):
        return jax.random.permutation(self._next(), n)
kernel_name = 'adaLN_cond__sliding_block_cached__moe_arch_mod__prompt'

def setup_inputs():
    _rng = _Rng(jax.random.key(int.from_bytes(__import__("os").urandom(4), "little")))
    _w = lambda a: (lambda t: t.astype(jnp.bfloat16) if jnp.issubdtype(t.dtype, jnp.floating) else t)(jnp.asarray(a))

    def _A_setup():
        B, Sq, D = (1, 2048, 1024)
        Hq, Hkv, Sk, Dh = (32, 4, 2048, 128)
        assert Hq % Hkv == 0, (Hq, Hkv)
        return {'x': _w((lambda *s: _rng.normal(s) * 0.05)(B, Sq, D)), 'k_cache': _w((lambda *s: _rng.normal(s) * 0.05)(B, Hkv, Sk, Dh)), 'v_cache': _w((lambda *s: _rng.normal(s) * 0.05)(B, Hkv, Sk, Dh)), 'wq': _w((lambda *s: _rng.normal(s) * 0.05)(D, Hq * Dh) * D ** (-0.5)), 'wo': _w((lambda *s: _rng.normal(s) * 0.05)(Hq * Dh, D) * (Hq * Dh) ** (-0.5))}
    _A_in = _A_setup()

    def _B_setup():
        B, S, D, F, C = (1, 2048, 1024, 3584, 1)
        return {'x': _w((lambda *s: _rng.normal(s) * 0.05)(B, S, D)), 'w_r': _w((lambda *s: _rng.normal(s) * 0.05)(D)), 'w_gate': _w((lambda *s: _rng.normal(s) * 0.05)(D, F)), 'w_up': _w((lambda *s: _rng.normal(s) * 0.05)(D, F)), 'w_down': _w((lambda *s: _rng.normal(s) * 0.05)(F, D))}
    _B_in = _B_setup()
    return {'A_x': _A_in['x'], 'A_k_cache': _A_in['k_cache'], 'A_v_cache': _A_in['v_cache'], 'A_wq': _A_in['wq'], 'A_wo': _A_in['wo'], 'B_x': _B_in['x'], 'B_w_r': _B_in['w_r'], 'B_w_gate': _B_in['w_gate'], 'B_w_up': _B_in['w_up'], 'B_w_down': _B_in['w_down'], 'c': _w((lambda *s: _rng.normal(s) * 0.05)(1, 1024)), 'w_mod': _w((lambda *s: _rng.normal(s) * 0.05)(1024, 6 * 1024) * 1024 ** (-0.5))}

def reference(A_x, A_k_cache, A_v_cache, A_wq, A_wo, B_x, B_w_r, B_w_gate, B_w_up, B_w_down, c, w_mod):

    def _A_ref(x, k_cache, v_cache, wq, wo):
        B, Sq, D = x.shape
        Hq, Dh = (32, 128)
        Hkv, Sk = (k_cache.shape[1], k_cache.shape[2])
        W = min(4096, max(256, Sk // 4))
        rep = Hq // Hkv
        q = (lambda x, *d: x.transpose(*d))((x @ wq).reshape(B, Sq, Hq, Dh), 0, 2, 1, 3)
        k = jnp.repeat(k_cache[:, :, Sk - W:, :], rep, axis=1)
        v = jnp.repeat(v_cache[:, :, Sk - W:, :], rep, axis=1)
        scores = jnp.einsum('bhqd,bhkd->bhqk', q, k) * Dh ** (-0.5)
        p = _softmax(scores, axis=-1)
        o = jnp.einsum('bhqk,bhkd->bhqd', p, v)
        return (lambda x, *d: x.transpose(*d))(o, 0, 2, 1, 3).reshape(B, Sq, Hq * Dh) @ wo

    def _B_ref(x, w_r, w_gate, w_up, w_down):
        B, S, D = x.shape
        C = 1
        r = x @ w_r
        idx = jnp.argsort(-r, axis=-1)[:, :C]
        idx_e = jnp.repeat(idx.reshape(B, C, 1), D, axis=2)
        x_sel = jnp.take_along_axis(x, idx_e, axis=1)
        g = _silu(x_sel @ w_gate)
        u = x_sel @ w_up
        y = g * u @ w_down
        r_sel = _sigmoid(jnp.take_along_axis(r, idx, axis=1))
        y = y * r_sel.reshape(B, C, 1)
        b_off = (jnp.arange(B) * S).reshape(B, 1)
        flat_idx = (idx + b_off).reshape(B * C)
        zero = (x * 0.0).reshape(B * S, D)
        upd = _scatter_add(zero, flat_idx, y.reshape(B * C, D), axis=0)
        return x + upd.reshape(B, S, D)
    x = A_x
    mod = (_silu(c) @ w_mod).reshape(c.shape[0], 6, 1, -1)
    sa, ca, ga, sb, cb, gb = (mod[:, 0].copy(), mod[:, 1].copy(), mod[:, 2].copy(), mod[:, 3].copy(), mod[:, 4].copy(), mod[:, 5].copy())
    h = _layernorm(x, axis=-1) * (1 + ca) + sa
    x = x + ga * _A_ref(h, A_k_cache, A_v_cache, A_wq, A_wo)
    h = _layernorm(x, axis=-1) * (1 + cb) + sb
    x = x + gb * _B_ref(h, B_w_r, B_w_gate, B_w_up, B_w_down)
    return x
```

```python
import jax
import jax.numpy as jnp
from jax import lax
import jax.experimental.pallas as pl
import jax.experimental.pallas.tpu as pltpu

S, D, HQ, HKV, DH, SK, W, F = 2048, 1024, 32, 4, 128, 2048, 512, 3584
REP = HQ // HKV
GW = REP * DH
TM = 512
NB = S // TM
QR = TM // HKV
SR = QR // 4
FENCE = True
ANCHOR_O = True
LOG2E = 1.4426950408889634
QSCALE = (DH ** -0.5) * LOG2E
EPS = 1e-5
f32, bf16, u32, i32 = jnp.float32, jnp.bfloat16, jnp.uint32, jnp.int32

S_C, S_WMS, S_WMC, S_X0, S_X2, S_WR, S_WG, S_WU, S_WD, S_FIN = range(10)
S_WQ = 10
S_WO = S_WQ + 2 * HKV
S_K = S_WO + HKV
S_V = S_K + HKV
S_X1 = S_V + HKV
S_WMB = S_X1 + HKV
S_OUT = S_WMB + 1
NSEM = S_OUT + NB


def _ln(x):
    m = jnp.mean(x, axis=-1, keepdims=True)
    xc = x - m
    v = jnp.mean(xc * xc, axis=-1, keepdims=True)
    return xc * lax.rsqrt(v + EPS)


def _pack(x):
    return pltpu.bitcast(x.astype(bf16), u32)


def _bf(x):
    return pltpu.bitcast(x, bf16)


def _mo(x, m):
    return x if isinstance(x, int) else pl.multiple_of(x, m)


def _recip(l):
    r = pl.reciprocal(l, approx=True)
    return r * (2.0 - l * r)


def _kernel(x_hbm, k_hbm, v_hbm, wq_hbm, wo_hbm, wr_hbm, wg_hbm, wu_hbm, wd_hbm, c_hbm, wm_hbm,
            out_hbm,
            x_v, k_v, v_v, wq_v, wo_v, wr_v, wg_v, wu_v, wd_v, c_v, wm_v,
            h_v, o_v, acc_v, out_v, x1_v, mod_v, best_v, besti_v, zero_v, zs_ref, sems):
    def cp(src, dst, i):
        return pltpu.make_async_copy(src, dst.bitcast(bf16), sems.at[i])

    def cp_rows(hbm, vm, r0, n, i):
        return cp(hbm.at[pl.ds(_mo(r0, n), n), :], vm.at[pl.ds(_mo(r0 // 2, n // 2), n // 2), :], i)

    def cp_cols(hbm, vm, c0, n, i):
        return cp(hbm.at[:, pl.ds(_mo(c0, 128), n)], vm.at[:, pl.ds(_mo(c0, 128), n)], i)

    def cp_wq(g, half):
        return cp_cols(wq_hbm, wq_v, g * GW + half * (GW // 2), GW // 2, S_WQ + 2 * g + half)

    def cp_k(g):
        return cp(k_hbm.at[g, pl.ds(SK - W, W), :], k_v.at[g], S_K + g)

    def cp_v(g):
        return cp(v_hbm.at[g, pl.ds(SK - W, W), :], v_v.at[g], S_V + g)

    def cp_x1(g):
        return cp_rows(x_hbm, x_v, TM + g * QR, QR, S_X1 + g)


    def cp_wo(g):
        return cp_rows(wo_hbm, wo_v, g * GW, GW, S_WO + g)

    def cp_out(i):
        r0 = i * TM
        return pltpu.make_async_copy(out_v.at[pl.ds(_mo(r0 // 2, TM // 2), TM // 2), :].bitcast(bf16),
                                     out_hbm.at[pl.ds(_mo(r0, TM), TM), :], sems.at[S_OUT + i])

    cp_c = pltpu.make_async_copy(c_hbm, c_v, sems.at[S_C])
    cp_wr = pltpu.make_async_copy(wr_hbm, wr_v, sems.at[S_WR])
    cp_wms = cp_cols(wm_hbm, wm_v, 0, D, S_WMS)
    cp_wmc = cp_cols(wm_hbm, wm_v, D, D, S_WMC)
    cp_wmb = cp_cols(wm_hbm, wm_v, 2 * D, 4 * D, S_WMB)
    cp_x0 = cp_rows(x_hbm, x_v, 0, TM, S_X0)
    cp_x2 = cp_rows(x_hbm, x_v, 2 * TM, S - 2 * TM, S_X2)
    cp_wg = cp(wg_hbm, wg_v, S_WG)
    cp_wu = cp(wu_hbm, wu_v, S_WU)
    cp_wd = cp(wd_hbm, wd_v, S_WD)

    for d in (cp_c, cp_x0, cp_wms, cp_wmc):
        d.start()
    for g in range(HKV):
        for d in (cp_wq(g, 0), cp_x1(g), cp_wq(g, 1), cp_k(g), cp_v(g), cp_wo(g)):
            d.start()
    for d in (cp_wmb, cp_wr, cp_x2, cp_wg, cp_wu, cp_wd):
        d.start()
    best_v[...] = jnp.full(best_v.shape, -jnp.inf, f32)
    besti_v[...] = jnp.zeros(besti_v.shape, i32)
    zero_v[...] = jnp.zeros(zero_v.shape, u32)
    mod_v[...] = jnp.zeros(mod_v.shape, f32)
    zs_ref[0] = 0
    cp_c.wait()
    cc = c_v[...].astype(f32)
    sc = jnp.broadcast_to((cc * jax.nn.sigmoid(cc)).astype(bf16), (16, D))
    cp_x0.wait()
    acc_v[1] = _ln(_bf(x_v[0:TM // 2, :]).astype(f32))
    cp_wms.wait()
    mod_v[:, 0:D] = jnp.dot(sc, _bf(wm_v[:, 0:D]), preferred_element_type=f32)[0:8]
    cp_wmc.wait()
    mod_v[:, D:2 * D] = jnp.dot(sc, _bf(wm_v[:, D:2 * D]), preferred_element_type=f32)[0:8]
    h_v[0] = _pack(acc_v[1] * (1.0 + mod_v[0:1, D:2 * D]) + mod_v[0:1, 0:D])

    def ln1_rows(row0, nrows, slot, dst0):
        sa = mod_v[0:1, 0 * D:1 * D]
        ca = mod_v[0:1, 1 * D:2 * D]
        xb = _bf(x_v[pl.ds(_mo(row0 // 2, nrows // 2), nrows // 2), :]).astype(f32)
        h = _ln(xb) * (1.0 + ca) + sa
        h_v[slot, pl.ds(_mo(dst0, nrows // 2), nrows // 2), :] = _pack(h)

    def epi_rows(src_row0, dst_row0, nrows, slot, acc0):
        ga = mod_v[0:1, 2 * D:3 * D]
        sb = mod_v[0:1, 3 * D:4 * D]
        cb = mod_v[0:1, 4 * D:5 * D]
        gb = mod_v[0:1, 5 * D:6 * D]
        wr = wr_v[...].astype(f32).reshape(1, D)
        src = pl.ds(_mo(src_row0 // 2, nrows // 2), nrows // 2)
        dst = pl.ds(_mo(dst_row0 // 2, nrows // 2), nrows // 2)
        x1 = _bf(x_v[src, :]).astype(f32) + ga * acc_v[slot, pl.ds(_mo(acc0, nrows), nrows), :]
        x1_v[dst, :] = _pack(x1)
        h2 = _ln(x1) * (1.0 + cb) + sb
        out_v[dst, :] = _pack(x1 + gb * h2)
        return jnp.sum(h2 * wr, axis=-1, keepdims=True)

    def upd_best(r, row0, nrows, pos0, valid=None):
        rb = jnp.broadcast_to(r, (nrows, 128))
        ib = row0 + lax.broadcasted_iota(i32, (nrows, 128), 0)
        sl = pl.ds(pos0, nrows)
        better = rb > best_v[sl, :]
        if valid is not None:
            better = better & valid
        best_v[sl, :] = jnp.where(better, rb, best_v[sl, :])
        besti_v[sl, :] = jnp.where(better, ib, besti_v[sl, :])

    def period(i, g, first):
        c0 = g * GW
        hs = i % 2
        if not first:
            @pl.when(i == 0)
            def _():
                for d in (cp_wq(g, 0), cp_x1(g), cp_wq(g, 1), cp_k(g), cp_v(g), cp_wo(g)):
                    d.wait()

            @pl.when((g == 0) & (i >= 2))
            def _():
                cp_out(i - 2).start()

        zero = zero_v[...]
        zs = zs_ref[0]

        def anchored(w, tok):
            if tok is None:
                return w
            wu = pltpu.bitcast(w, u32)
            wu = jnp.concatenate([wu[0:8, :] | jnp.tile(tok & zero, (1, wu.shape[1] // 128)), wu[8:, :]], axis=0)
            return pltpu.bitcast(wu, bf16)

        def side(j, dz):
            sub = j // 2
            q0 = g * QR + sub * SR
            if j % 2 == 0:
                if first:
                    return None
                src0 = jnp.maximum(i - 1, 0) * TM + q0 + dz
                dst0 = jnp.where(i == 0, S, (i - 1) * TM) + q0 + dz
                r = epi_rows(src0, dst0, SR, 1 - hs, q0 + dz)
                upd_best(r, dst0, SR, sub * SR, i > 0)
                opq = pl.ds(pl.multiple_of(dst0 // 2 + zs, 8), 8)
                ob = pl.ds(pl.multiple_of(sub * SR + zs, 8), 8)
                return (out_v[opq, 0:128] | x1_v[opq, 0:128]
                        | pltpu.bitcast(best_v[ob, :], u32) | pltpu.bitcast(besti_v[ob, :], u32))
            else:
                if first and j == 1:
                    cp_x1(0).wait()
                ln1_rows(jnp.minimum(i + 1, NB - 1) * TM + q0 + dz, SR, 1 - hs, q0 // 2)
                return h_v[1 - hs, pl.ds(pl.multiple_of(q0 // 2 + zs, 8), 8), 0:128]

        h = _bf(h_v[hs])
        qs = []
        toks = [None, None]
        for hh in range(REP):
            if first and hh % (REP // 2) == 0:
                cp_wq(0, hh // (REP // 2)).wait()
            w = anchored(_bf(wq_v[:, pl.ds(pl.multiple_of(c0 + hh * DH, DH), DH)]), toks[hh])
            qh = jnp.dot(h, w, preferred_element_type=f32)
            qs.append((qh * QSCALE).astype(bf16))
            dz = 0
            if FENCE:
                dz = pltpu.bitcast(qh[0:8, 0:128], i32)[0, 0] & zs
            toks.append(side(hh, dz))
        if first:
            cp_k(0).wait()
            cp_v(0).wait()
        kk = _bf(k_v[g])
        vv = _bf(v_v[g])
        otok = None
        for hh in range(REP):
            s = lax.dot_general(qs[hh], anchored(kk, toks[REP + hh]) if hh < 2 else kk,
                                (((1,), (1,)), ((), ())), preferred_element_type=f32)
            m = jnp.max(s, axis=-1, keepdims=True)
            p = jnp.exp2(s - m)
            l = jnp.sum(p, axis=-1, keepdims=True)
            o = jnp.dot(p.astype(bf16), anchored(vv, otok), preferred_element_type=f32)
            o_v[:, hh * DH:(hh + 1) * DH] = _pack(o * _recip(l))
            if ANCHOR_O and hh + 2 < REP:
                otok = o_v[pl.ds(pl.multiple_of(zs, 8), 8), pl.ds(pl.multiple_of(hh * DH + zs * 128, DH), DH)]
        if first:
            cp_wo(0).wait()
        contrib = jnp.dot(_bf(o_v[...]), _bf(wo_v[pl.ds(pl.multiple_of(c0 // 2, GW // 2), GW // 2), :]),
                          preferred_element_type=f32)
        acc_v[hs] = jnp.where(g == 0, contrib, acc_v[hs] + contrib)
        if not first:
            @pl.when((i == 0) & (g == HKV - 1))
            def _():
                cp_wmb.wait()
                cp_wr.wait()
                cp_x2.wait()
                mod_v[:, 2 * D:6 * D] = jnp.dot(sc, _bf(wm_v[:, 2 * D:6 * D]), preferred_element_type=f32)[0:8]

    with jax.named_scope("p00"):
        period(0, 0, True)
    with jax.named_scope("loop"):
        def step(t, _):
            period(t // HKV, t % HKV, False)
        lax.fori_loop(1, NB * HKV, step, None)
    cp_out(NB - 2).start()

    with jax.named_scope("tail"):
        r = epi_rows((NB - 1) * TM, (NB - 1) * TM, TM, (NB - 1) % 2, 0)
        cp_out(NB - 1).start()
        for qd in range(HKV):
            upd_best(r[qd * QR:(qd + 1) * QR], (NB - 1) * TM + qd * QR, QR, 0)
        bv = best_v[...]
        mx = jnp.max(bv)
        idx = jnp.min(jnp.where(bv == mx, besti_v[...], S))
        idx = jnp.minimum(idx, S - 1)
        base = pl.multiple_of((idx // 16) * 16, 16)
        pb = pl.ds(pl.multiple_of(base // 2, 8), 8)
        sb = mod_v[0:1, 3 * D:4 * D]
        cb = mod_v[0:1, 4 * D:5 * D]
        gb = mod_v[0:1, 5 * D:6 * D]
        wr = wr_v[...].astype(f32).reshape(1, D)
        x1 = _bf(x1_v[pb, :]).astype(f32)
        h2 = _ln(x1) * (1.0 + cb) + sb
        hsel = h2.astype(bf16)
        r_sel = jnp.sum(hsel.astype(f32) * wr, axis=-1, keepdims=True)
        cp_wg.wait()
        gg = jnp.dot(hsel, _bf(wg_v[...]), preferred_element_type=f32)
        cp_wu.wait()
        uu = jnp.dot(hsel, _bf(wu_v[...]), preferred_element_type=f32)
        a = (gg * jax.nn.sigmoid(gg) * uu).astype(bf16)
        cp_wd.wait()
        y = jnp.dot(a, _bf(wd_v[...]), preferred_element_type=f32)
        y = y * jax.nn.sigmoid(r_sel)
        rows = base + lax.broadcasted_iota(i32, (16, D), 0)
        new = (x1 + gb * (h2 + y)).astype(bf16)
        for i in range(NB):
            cp_out(i).wait()
        out_v[pb, :] = pltpu.bitcast(jnp.where(rows == idx, new, _bf(out_v[pb, :])), u32)
        fin = pltpu.make_async_copy(out_v.at[pb, :].bitcast(bf16), out_hbm.at[pl.ds(base, 16), :], sems.at[S_FIN])
        fin.start()
        fin.wait()


@jax.jit
def pallas_adaLN_cond__sliding_block_cached__moe_arch_mod__prompt_kernel(
    A_x, A_k_cache, A_v_cache, A_wq, A_wo, B_x, B_w_r, B_w_gate, B_w_up, B_w_down, c, w_mod,
):
    anyspec = pl.BlockSpec(memory_space=pl.ANY)
    out = pl.pallas_call(
        _kernel,
        out_shape=jax.ShapeDtypeStruct((S, D), bf16),
        in_specs=[anyspec] * 11,
        out_specs=anyspec,
        scratch_shapes=[
            pltpu.VMEM((S // 2, D), u32),
            pltpu.VMEM((HKV, W // 2, DH), u32),
            pltpu.VMEM((HKV, W // 2, DH), u32),
            pltpu.VMEM((D // 2, HQ * DH), u32),
            pltpu.VMEM((HQ * DH // 2, D), u32),
            pltpu.VMEM((D,), bf16),
            pltpu.VMEM((D // 2, F), u32),
            pltpu.VMEM((D // 2, F), u32),
            pltpu.VMEM((F // 2, D), u32),
            pltpu.VMEM((1, D), bf16),
            pltpu.VMEM((D // 2, 6 * D), u32),
            pltpu.VMEM((2, TM // 2, D), u32),
            pltpu.VMEM((TM // 2, GW), u32),
            pltpu.VMEM((2, TM, D), f32),
            pltpu.VMEM((S // 2 + TM // 2, D), u32),
            pltpu.VMEM((S // 2 + TM // 2, D), u32),
            pltpu.VMEM((8, 6 * D), f32),
            pltpu.VMEM((QR, 128), f32),
            pltpu.VMEM((QR, 128), i32),
            pltpu.VMEM((8, 128), u32),
            pltpu.SMEM((1,), i32),
            pltpu.SemaphoreType.DMA((NSEM,)),
        ],
        compiler_params=pltpu.CompilerParams(vmem_limit_bytes=100 * 1024 * 1024),
    )(
        A_x.reshape(S, D), A_k_cache.reshape(HKV, SK, DH), A_v_cache.reshape(HKV, SK, DH),
        A_wq, A_wo, B_w_r, B_w_gate, B_w_up, B_w_down, c, w_mod,
    )
    return out.reshape(1, S, D)
```

```python
import jax
import jax.numpy as jnp
from jax import lax
import jax.experimental.pallas as pl
import jax.experimental.pallas.tpu as pltpu

S, D, HQ, HKV, DH, SK, W, F = 2048, 1024, 32, 4, 128, 2048, 512, 3584
REP = HQ // HKV
GW = REP * DH
TM = 512
NB = S // TM
QR = TM // HKV
HM = TM // 2
HK = D // 2
WPARTS = 4 * D // DH // HKV
SIDE_STRIDE = 6
SIDE_DIST = 4
PREP_UNROLL = 1
CR = 32
SR = 16
NSL = HM // HKV // SR
FENCE = True
ANCHOR_O = True
LOG2E = 1.4426950408889634
QSCALE = (DH ** -0.5) * LOG2E
EPS = 1e-5
f32, bf16, u32, i32 = jnp.float32, jnp.bfloat16, jnp.uint32, jnp.int32

S_C, S_WMS, S_WMC, S_X0, S_X2, S_WR, S_FIN = range(7)
S_WQ = 7
S_WO = S_WQ + 2 * HKV
S_K = S_WO + HKV
S_V = S_K + HKV
S_X1 = S_V + HKV
S_WMB = S_X1 + 2 * HKV
S_OUT = S_WMB + HKV
NFP = 7
FP = F // NFP
S_WG = S_OUT + NB
S_WU = S_WG + NFP
S_WD = S_WU + NFP
NSEM = S_WD + NFP


def _ln(x):
    m = jnp.mean(x, axis=-1, keepdims=True)
    xc = x - m
    v = jnp.mean(xc * xc, axis=-1, keepdims=True)
    return xc * lax.rsqrt(v + EPS)


def _packs(y):
    r, c = y.shape
    y4 = y.reshape(r // 16, 2, 8, c)
    return pltpu.pack_elementwise([y4[:, 0].reshape(r // 2, c), y4[:, 1].reshape(r // 2, c)], packed_dtype=bf16)


def _halves(w):
    return tuple(pltpu.unpack_elementwise(w, index=n, packed_dtype=bf16, unpacked_dtype=f32) for n in range(2))


def _unpacks(w):
    r, c = w.shape
    lo, hi = (t.reshape(r // 8, 8, c) for t in _halves(w))
    return jnp.stack([lo, hi], axis=1).reshape(2 * r, c)


def _bf(x):
    return pltpu.bitcast(x, bf16)


def _mo(x, m):
    return x if isinstance(x, int) else pl.multiple_of(x, m)


def _recip(l):
    r = pl.reciprocal(l, approx=True)
    return r * (2.0 - l * r)


def _kernel(x_hbm, k_hbm, v_hbm, wq_hbm, wo_hbm, wr_hbm, wg_hbm, wu_hbm, wd_hbm, c_hbm, wm_hbm,
            out_hbm,
            x_v, k_v, v_v, wq_v, wo_v, wr_v, wg_v, wu_v, wd_v, c_v, wm_v,
            h_v, h7_v, o_v, o7_v, q_v, qp_v, ost_v, bq_v, bo_v, acc_v, out_v, x1_v, mod_v, best_v, besti_v, zero_v, zs_ref, sems):
    def cp(src, dst, i):
        return pltpu.make_async_copy(src, dst.bitcast(bf16), sems.at[i])

    def cp_rows(hbm, vm, r0, n, i):
        return cp(hbm.at[pl.ds(_mo(r0, n), n), :], vm.at[pl.ds(_mo(r0 // 2, n // 2), n // 2), :], i)

    def cp_cols(hbm, vm, c0, n, i):
        return cp(hbm.at[:, pl.ds(_mo(c0, 128), n)], vm.at[:, pl.ds(_mo(c0, 128), n)], i)

    def cp_wq(g, half):
        return cp_cols(wq_hbm, wq_v, g * GW + half * (GW // 2), GW // 2, S_WQ + 2 * g + half)

    def cp_k(g):
        return cp(k_hbm.at[g, pl.ds(SK - W, W), :], k_v.at[g], S_K + g)

    def cp_v(g):
        return cp(v_hbm.at[g, pl.ds(SK - W, W), :], v_v.at[g], S_V + g)

    def cp_x1(g, half):
        n = HM // HKV
        return cp_rows(x_hbm, x_v, TM + half * HM + g * n, n, S_X1 + 2 * g + half)


    def cp_wo(g):
        return cp_rows(wo_hbm, wo_v, g * GW, GW, S_WO + g)

    def cp_out(i):
        r0 = i * TM
        return pltpu.make_async_copy(out_v.at[pl.ds(_mo(r0 // 2, TM // 2), TM // 2), :].bitcast(bf16),
                                     out_hbm.at[pl.ds(_mo(r0, TM), TM), :], sems.at[S_OUT + i])

    cp_c = pltpu.make_async_copy(c_hbm, c_v, sems.at[S_C])
    cp_wr = pltpu.make_async_copy(wr_hbm, wr_v, sems.at[S_WR])
    cp_wms = cp_cols(wm_hbm, wm_v, 0, D, S_WMS)
    cp_wmc = cp_cols(wm_hbm, wm_v, D, D, S_WMC)
    cp_x0 = cp_rows(x_hbm, x_v, 0, TM, S_X0)
    cp_x2 = cp_rows(x_hbm, x_v, 2 * TM, S - 2 * TM, S_X2)

    def cp_wmb(n):
        return cp_cols(wm_hbm, wm_v, (2 + n) * D, D, S_WMB + n)

    def cp_ffn(n):
        return (cp_cols(wg_hbm, wg_v, n * FP, FP, S_WG + n), cp_cols(wu_hbm, wu_v, n * FP, FP, S_WU + n),
                cp_rows(wd_hbm, wd_v, n * FP, FP, S_WD + n))

    def group_set(g):
        return (cp_wq(g, 0), cp_x1(g, 0), cp_x1(g, 1), cp_wq(g, 1), cp_k(g), cp_v(g), cp_wo(g))


    for d in (cp_c, cp_x0, cp_wms, cp_wmc) + group_set(0):
        d.start()
    best_v[...] = jnp.full(best_v.shape, -jnp.inf, f32)
    besti_v[...] = jnp.zeros(besti_v.shape, i32)
    zero_v[...] = jnp.zeros(zero_v.shape, u32)
    mod_v[...] = jnp.zeros(mod_v.shape, f32)
    for n in range(8):
        zs_ref[n] = 0
    cp_c.wait()
    cc = c_v[...].astype(f32)
    sc = jnp.broadcast_to((cc * jax.nn.sigmoid(cc)).astype(bf16), (16, D))
    cp_x0.wait()
    acc_v[1] = _ln(_bf(x_v[0:TM // 2, :]).astype(f32))
    cp_wms.wait()
    mod_v[:, 0:D] = jnp.dot(sc, _bf(wm_v[:, 0:D]), preferred_element_type=f32)[0:8]
    cp_wmc.wait()
    mod_v[:, D:2 * D] = jnp.dot(sc, _bf(wm_v[:, D:2 * D]), preferred_element_type=f32)[0:8]
    h_v[...] = _packs(acc_v[1] * (1.0 + mod_v[0:1, D:2 * D]) + mod_v[0:1, 0:D])

    def ln1_slice(row0, slot, dst0, normed=False):
        sa = mod_v[0:1, 0 * D:1 * D]
        ca1 = 1.0 + mod_v[0:1, 1 * D:2 * D]
        if normed:
            xt, xb = acc_v[1, row0:row0 + 16, :], acc_v[1, row0 + HM:row0 + HM + 16, :]
            norm = lambda t: t
        else:
            xt = _bf(x_v[pl.ds(_mo(row0 // 2, 8), 8), :]).astype(f32)
            xb = _bf(x_v[pl.ds(_mo((row0 + HM) // 2, 8), 8), :]).astype(f32)
            norm = _ln
        dst = pl.ds(_mo(dst0 // 2, 8), 8)
        hs_ = []
        for r in (0, 8):
            top = norm(xt[r:r + 8]) * ca1 + sa
            bot = norm(xb[r:r + 8]) * ca1 + sa
            a11, a12, a21, a22 = top[:, :HK], top[:, HK:], bot[:, :HK], bot[:, HK:]
            hs_.append((a11 + a22, a21 + a22, a11, a22, a11 + a12, a21 - a11, a12 - a22))
        for n in range(7):
            h7_v[slot, n, dst, :] = pltpu.pack_elementwise([hs_[0][n], hs_[1][n]], packed_dtype=bf16)

    def wsum_slice(halves, dst):
        nr = dst.shape[1]
        for rr in range(0, nr, 8):
            for c in range(0, HK, 128):
                b11, b12, b21, b22 = (_halves(halves[kh][rr:rr + 8, nh * HK + c:nh * HK + c + 128])
                                      for kh in range(2) for nh in range(2))
                for n, (p, q, sign) in enumerate(((b11, b22, 1), (b12, b22, -1), (b21, b11, -1),
                                                  (b11, b12, 1), (b21, b22, 1))):
                    dst[n, rr:rr + 8, c:c + 128] = pltpu.pack_elementwise(
                        [u + w if sign > 0 else u - w for u, w in zip(p, q)], packed_dtype=bf16)

    def epi_rows(src_row0, dst_row0, nrows, slot, acc0):
        ga = mod_v[0:1, 2 * D:3 * D]
        sb = mod_v[0:1, 3 * D:4 * D]
        cb = mod_v[0:1, 4 * D:5 * D]
        gb = mod_v[0:1, 5 * D:6 * D]
        wr = wr_v[...].astype(f32).reshape(1, D)
        src = pl.ds(_mo(src_row0 // 2, nrows // 2), nrows // 2)
        dst = pl.ds(_mo(dst_row0 // 2, nrows // 2), nrows // 2)
        x1 = _unpacks(x_v[src, :]) + ga * acc_v[slot, pl.ds(_mo(acc0, nrows), nrows), :]
        x1_v[dst, :] = _packs(x1)
        h2 = _ln(x1) * (1.0 + cb) + sb
        out_v[dst, :] = _packs(x1 + gb * h2)
        return jnp.sum(h2 * wr, axis=-1, keepdims=True)

    def epi_rows16(src0, row0, slot, acc0, pos0, valid):
        ga = mod_v[0:1, 2 * D:3 * D]
        sb = mod_v[0:1, 3 * D:4 * D]
        cb1 = 1.0 + mod_v[0:1, 4 * D:5 * D]
        gb = mod_v[0:1, 5 * D:6 * D]
        wr = wr_v[...].astype(f32).reshape(1, D)
        rows = pl.ds(_mo(row0 // 2, 8), 8)
        xs = _halves(x_v[pl.ds(_mo(src0 // 2, 8), 8), :])
        x1s, outs = [], []
        for n in range(2):
            x1 = xs[n] + ga * acc_v[slot, pl.ds(_mo(acc0 + 8 * n, 8), 8), :]
            h2 = _ln(x1) * cb1 + sb
            x1s.append(x1)
            outs.append(x1 + gb * h2)
            r = jnp.broadcast_to(jnp.sum(h2 * wr, axis=-1, keepdims=True), (8, 128))
            ib = row0 + n + 2 * lax.broadcasted_iota(i32, (8, 128), 0)
            sl = pl.ds(pos0 + 8 * n, 8)
            better = (r > best_v[sl, :]) & valid
            best_v[sl, :] = jnp.where(better, r, best_v[sl, :])
            besti_v[sl, :] = jnp.where(better, ib, besti_v[sl, :])
        x1_v[rows, :] = pltpu.pack_elementwise(x1s, packed_dtype=bf16)
        out_v[rows, :] = pltpu.pack_elementwise(outs, packed_dtype=bf16)

    def upd_best(r, row0, nrows, pos0, valid=None):
        rb = jnp.broadcast_to(r, (nrows, 128))
        p = lax.broadcasted_iota(i32, (nrows, 128), 0)
        ib = row0 + (p & ~15) + 2 * (p & 7) + ((p & 15) >> 3)
        sl = pl.ds(pos0, nrows)
        better = rb > best_v[sl, :]
        if valid is not None:
            better = better & valid
        best_v[sl, :] = jnp.where(better, rb, best_v[sl, :])
        besti_v[sl, :] = jnp.where(better, ib, besti_v[sl, :])

    def wq_quad(g):
        def quad(kh, nh, r0=0, nr=HK // 2, c=0, nc=HK):
            return wq_v[pl.ds(_mo(kh * (HK // 2) + r0, 8), nr), pl.ds(_mo(g * GW + nh * HK + c, DH), nc)]
        return quad

    def wo_quad(g):
        def quad(kh, nh, r0=0, nr=HK // 2, c=0, nc=HK):
            return wo_v[pl.ds(_mo((g * GW + kh * HK) // 2 + r0, 8), nr), pl.ds(_mo(nh * HK + c, DH), nc)]
        return quad

    def b_operand(quad, sums, g, n, j):
        if n == 1:
            return quad(0, 0, c=j * DH, nc=DH)
        if n == 4:
            return quad(1, 1, c=j * DH, nc=DH)
        return sums[g, (0, None, 1, 2, None, 3, 4)[n], :, j * DH:(j + 1) * DH]

    def prep(g):
        def body(part, _):
            nr = HK // 2 // WPARTS
            r0 = part * nr
            rows = pl.ds(pl.multiple_of(r0, nr), nr)
            wsum_slice([wq_v.at[pl.ds(pl.multiple_of(kh * (HK // 2) + r0, nr), nr),
                                pl.ds(pl.multiple_of(g * GW, GW), GW)] for kh in range(2)], bq_v.at[g, :, rows, :])
            wsum_slice([wo_v.at[pl.ds(pl.multiple_of((g * GW + kh * HK) // 2 + r0, nr), nr), :]
                        for kh in range(2)], bo_v.at[g, :, rows, :])
        lax.fori_loop(0, WPARTS, body, None)

    def period(i, g, mode):
        hs = i % 2
        if mode == 2:
            @pl.when(i == 0)
            def _():
                @pl.when(g < HKV - 1)
                def _():
                    for d in group_set(g + 1):
                        d.start()

                @pl.when(g == HKV - 1)
                def _():
                    cp_wr.start()
                    cp_x2.start()
                cp_wmb(g).start()
                for d in group_set(g):
                    d.wait()
                prep(g)

            @pl.when((i == 1) & (g == 0))
            def _():
                for n in range(HKV):
                    cp_wmb(n).wait()
                cp_wr.wait()
                cp_x2.wait()
                prep(0)
                mod_v[:, 2 * D:6 * D] = jnp.dot(sc, _bf(wm_v[:, 2 * D:6 * D]), preferred_element_type=f32)[0:8]

            @pl.when((g == 0) & (i >= 2))
            def _():
                cp_out(i - 2).start()

            piece = i * HKV + g - HKV

            @pl.when((piece >= 0) & (piece < NFP))
            def _():
                for d in cp_ffn(piece):
                    d.start()

        zero = zero_v[...]
        zz = [zs_ref[n] for n in range(8)]
        zs = zz[0]

        def ln_work(sub, dz):
            if mode == 0 and sub == 0:
                cp_x1(0, 0).wait()
                cp_x1(0, 1).wait()
            q0 = g * (HM // HKV) + sub * SR
            ln1_slice(jnp.minimum(i + 1, NB - 1) * TM + q0 + dz, 1 - hs, q0)
            return h7_v[1 - hs, 0, pl.ds(pl.multiple_of(q0 // 2 + zs, 8), 8), 0:128]

        def epi_work(sub, dz):
            toks = None
            for half in range(2):
                q0 = half * HM + g * (HM // HKV) + sub * SR
                src0 = jnp.maximum(i - 1, 0) * TM + q0
                row0 = jnp.where(i == 0, S, (i - 1) * TM) + q0
                pos = (2 * sub + half) * SR
                epi_rows16(src0, row0, 1 - hs, q0, pos, i > 0)
                opq = pl.ds(pl.multiple_of(row0 // 2 + zs, 8), 8)
                ob = pl.ds(pl.multiple_of(pos + zs, 8), 8)
                t = (out_v[opq, 0:128] | x1_v[opq, 0:128]
                     | pltpu.bitcast(best_v[ob, :], u32) | pltpu.bitcast(besti_v[ob, :], u32))
                toks = t if toks is None else toks | t
            return toks

        early, late = [], []
        if mode == 2:
            for sub in range(NSL):
                early += [lambda dz, sub=sub: epi_work(sub, dz)] + [None] * (SIDE_STRIDE - 1)
                late += [lambda dz, sub=sub: ln_work(sub, dz)] + [None] * (SIDE_STRIDE - 1)
        else:
            def h7_first(n):
                ln1_slice(n * SR, 0, n * SR, normed=True)
                return h7_v[0, 0, pl.ds(pl.multiple_of(n * (SR // 2) + zs, 8), 8), 0:128]
            for sub in range(NSL):
                early.append(lambda dz, sub=sub: ln_work(sub, dz))
            for n in range(HM // SR):
                early.append(lambda dz, n=n: h7_first(n))
        pending = [None] * (SIDE_DIST if mode == 2 else 2)

        def anchored(w, extra=None):
            tok = pending.pop(0) if pending else None
            if extra is not None:
                tok = extra if tok is None else tok | extra
            if tok is not None:
                w = jnp.concatenate([w[0:8, :] | jnp.tile(tok & zero, (1, w.shape[1] // 128)), w[8:, :]], axis=0)
            return _bf(w)

        def after(res, queue):
            work = queue.pop(0) if queue else None
            if work is not None:
                pending.append(work(0))
            else:
                pending.append(None)

        def mm(a, w, queue, extra=None):
            res = jnp.dot(a, anchored(w, extra), preferred_element_type=f32)
            after(res, queue)
            return res

        if mode == 0:
            for hh in range(REP):
                if hh % (REP // 2) == 0:
                    cp_wq(0, hh // (REP // 2)).wait()
                h = _bf(h_v[pl.ds(pl.multiple_of(zz[hh], 8), TM // 2), :])
                qh = mm(h, wq_v[:, pl.ds(_mo(g * GW + hh * DH, DH), DH)], early)
                q_v[:, hh * DH:(hh + 1) * DH] = _packs(qh * QSCALE)
        else:
            quad = wq_quad(g)
            for j in range(HK // DH):
                def d(n):
                    return mm(_bf(h7_v[hs + zz[j], n]), b_operand(quad, bq_v, g, n, j), early)
                L, R = pl.ds(0, DH), pl.ds(DH, DH)
                QL, QR_ = pl.ds(j * DH, DH), pl.ds(HK + j * DH, DH)
                def comb(m, *ops):
                    for r in range(0, HM, CR):
                        mc = m[r:r + CR]
                        for (row, col, kind, qsrc) in ops:
                            rows = pl.ds(row + r, CR)
                            if kind == "set":
                                qp_v[rows, col] = mc
                            elif kind == "add":
                                qp_v[rows, col] += mc
                            elif kind == "sub":
                                qp_v[rows, col] -= mc
                            else:
                                q_v[pl.ds((row + r) // 2, CR // 2), qsrc] = _packs((qp_v[rows, col] + mc) * QSCALE)
                comb(d(0), (0, L, "set", None), (HM, R, "set", None))
                comb(d(1), (HM, R, "sub", None), (HM, L, "set", None))
                comb(d(2), (HM, R, "add", None), (0, R, "set", None))
                comb(d(3), (0, L, "add", None), (HM, L, "q", QL))
                comb(d(4), (0, L, "sub", None), (0, R, "q", QR_))
                comb(d(5), (HM, R, "q", QR_))
                comb(d(6), (0, L, "q", QL))

        if mode == 0:
            cp_k(0).wait()
            cp_v(0).wait()
            for d in group_set(1) + (cp_wmb(0),):
                d.start()
        otok = None
        for hh in range(REP):
            s = lax.dot_general(_bf(q_v[:, hh * DH:(hh + 1) * DH]), anchored(k_v[g]), (((1,), (1,)), ((), ())), preferred_element_type=f32)
            after(s, early)
            m = jnp.max(s, axis=-1, keepdims=True)
            p = jnp.exp2(s - m)
            l = jnp.sum(p, axis=-1, keepdims=True)
            o = mm(p.astype(bf16), v_v[g], early, otok) * _recip(l)
            col = slice((hh % 4) * DH, (hh % 4 + 1) * DH)
            if mode != 2:
                o_v[:, hh * DH:(hh + 1) * DH] = _packs(o)
                oref = o_v
            elif hh < 4:
                top, bot = o[:HM], o[HM:]
                ost_v[:, col] = o
                o7_v[2, :, col] = _packs(top)
                o7_v[5, :, col] = _packs((bot - top))
                oref = o7_v.at[5]
            else:
                a12, a22 = o[:HM], o[HM:]
                a11, a21 = ost_v[0:HM, col], ost_v[HM:TM, col]
                o7_v[0, :, col] = _packs((a11 + a22))
                o7_v[1, :, col] = _packs((a21 + a22))
                o7_v[3, :, col] = _packs(a22)
                o7_v[4, :, col] = _packs((a11 + a12))
                o7_v[6, :, col] = _packs((a12 - a22))
                oref = o7_v.at[6]
            otok = None
            if hh + 2 < REP:
                cc = (hh * DH if mode != 2 else (hh % 4) * DH)
                otok = oref[pl.ds(pl.multiple_of(zs, 8), 8), pl.ds(pl.multiple_of(cc + zs * 128, DH), DH)]

        if mode == 0:
            cp_wo(0).wait()
        if mode != 2:
            for nt in range(D // DH):
                ob = _bf(o_v[pl.ds(pl.multiple_of(zz[nt], 8), TM // 2), :])
                cols = pl.ds(nt * DH, DH)
                contrib = mm(ob, wo_v[pl.ds(_mo(g * GW // 2, GW // 2), GW // 2), cols], late)
                acc_v[hs, :, cols] = contrib if mode == 0 else acc_v[hs, :, cols] + contrib
        else:
            quad = wo_quad(g)
            for j in range(HK // DH):
                def d(n):
                    return mm(_bf(o7_v[n + zz[j]]), b_operand(quad, bo_v, g, n, j), late)
                L, R = pl.ds(j * DH, DH), pl.ds(HK + j * DH, DH)

                def comb(m, *ops):
                    for r in range(0, HM, CR):
                        mc = m[r:r + CR]
                        for (row, col, kind) in ops:
                            rows = pl.ds(row + r, CR)
                            if kind == "first":
                                acc_v[hs, rows, col] = jnp.where(g == 0, mc, acc_v[hs, rows, col] + mc)
                            elif kind == "add":
                                acc_v[hs, rows, col] += mc
                            else:
                                acc_v[hs, rows, col] -= mc
                comb(d(0), (0, L, "first"), (HM, R, "first"))
                comb(d(1), (HM, R, "sub"), (HM, L, "first"))
                comb(d(2), (HM, R, "add"), (0, R, "first"))
                comb(d(3), (0, L, "add"), (HM, L, "add"))
                comb(d(4), (0, L, "sub"), (0, R, "add"))
                comb(d(5), (HM, R, "add"))
                comb(d(6), (0, L, "add"))
        assert not any(early) and not any(late)

    with jax.named_scope("p00"):
        period(0, 0, 0)
    with jax.named_scope("loopB"):
        def step_b(t, _):
            period(t // HKV, t % HKV, 2)
        lax.fori_loop(1, NB * HKV, step_b, None)
    cp_out(NB - 2).start()

    with jax.named_scope("tail"):
        r = epi_rows((NB - 1) * TM, (NB - 1) * TM, TM, (NB - 1) % 2, 0)
        cp_out(NB - 1).start()
        for qd in range(HKV):
            upd_best(r[qd * QR:(qd + 1) * QR], (NB - 1) * TM + qd * QR, QR, 0)
        bv = best_v[...]
        mx = jnp.max(bv)
        idx = jnp.min(jnp.where(bv == mx, besti_v[...], S))
        idx = jnp.minimum(idx, S - 1)
        base = pl.multiple_of((idx // 16) * 16, 16)
        pb = pl.ds(pl.multiple_of(base // 2, 8), 8)
        sb = mod_v[0:1, 3 * D:4 * D]
        cb = mod_v[0:1, 4 * D:5 * D]
        gb = mod_v[0:1, 5 * D:6 * D]
        wr = wr_v[...].astype(f32).reshape(1, D)
        x1 = _bf(x1_v[pb, :]).astype(f32)
        h2 = _ln(x1) * (1.0 + cb) + sb
        hsel = h2.astype(bf16)
        r_sel = jnp.sum(hsel.astype(f32) * wr, axis=-1, keepdims=True)
        for n in range(NFP):
            cp_cols(wg_hbm, wg_v, n * FP, FP, S_WG + n).wait()
        gg = jnp.dot(hsel, _bf(wg_v[...]), preferred_element_type=f32)
        for n in range(NFP):
            cp_cols(wu_hbm, wu_v, n * FP, FP, S_WU + n).wait()
        uu = jnp.dot(hsel, _bf(wu_v[...]), preferred_element_type=f32)
        a = (gg * jax.nn.sigmoid(gg) * uu).astype(bf16)
        for n in range(NFP):
            cp_rows(wd_hbm, wd_v, n * FP, FP, S_WD + n).wait()
        y = jnp.dot(a, _bf(wd_v[...]), preferred_element_type=f32)
        y = y * jax.nn.sigmoid(r_sel)
        rows = base + lax.broadcasted_iota(i32, (16, D), 0)
        new = (x1 + gb * (h2 + y)).astype(bf16)
        for i in range(NB):
            cp_out(i).wait()
        out_v[pb, :] = pltpu.bitcast(jnp.where(rows == idx, new, _bf(out_v[pb, :])), u32)
        fin = pltpu.make_async_copy(out_v.at[pb, :].bitcast(bf16), out_hbm.at[pl.ds(base, 16), :], sems.at[S_FIN])
        fin.start()
        fin.wait()


@jax.jit
def pallas_adaLN_cond__sliding_block_cached__moe_arch_mod__prompt_kernel(
    A_x, A_k_cache, A_v_cache, A_wq, A_wo, B_x, B_w_r, B_w_gate, B_w_up, B_w_down, c, w_mod,
):
    anyspec = pl.BlockSpec(memory_space=pl.ANY)
    out = pl.pallas_call(
        _kernel,
        out_shape=jax.ShapeDtypeStruct((S, D), bf16),
        in_specs=[anyspec] * 11,
        out_specs=anyspec,
        scratch_shapes=[
            pltpu.VMEM((S // 2, D), u32),
            pltpu.VMEM((HKV, W // 2, DH), u32),
            pltpu.VMEM((HKV, W // 2, DH), u32),
            pltpu.VMEM((D // 2, HQ * DH), u32),
            pltpu.VMEM((HQ * DH // 2, D), u32),
            pltpu.VMEM((D,), bf16),
            pltpu.VMEM((D // 2, F), u32),
            pltpu.VMEM((D // 2, F), u32),
            pltpu.VMEM((F // 2, D), u32),
            pltpu.VMEM((1, D), bf16),
            pltpu.VMEM((D // 2, 6 * D), u32),
            pltpu.VMEM((TM // 2, D), u32),
            pltpu.VMEM((2, 7, HM // 2, HK), u32),
            pltpu.VMEM((TM // 2, GW), u32),
            pltpu.VMEM((7, HM // 2, HK), u32),
            pltpu.VMEM((TM // 2, GW), u32),
            pltpu.VMEM((TM, 2 * DH), f32),
            pltpu.VMEM((TM, HK), f32),
            pltpu.VMEM((HKV, 5, HK // 2, HK), u32),
            pltpu.VMEM((HKV, 5, HK // 2, HK), u32),
            pltpu.VMEM((2, TM, D), f32),
            pltpu.VMEM((S // 2 + TM // 2, D), u32),
            pltpu.VMEM((S // 2 + TM // 2, D), u32),
            pltpu.VMEM((8, 6 * D), f32),
            pltpu.VMEM((QR, 128), f32),
            pltpu.VMEM((QR, 128), i32),
            pltpu.VMEM((8, 128), u32),
            pltpu.SMEM((8,), i32),
            pltpu.SemaphoreType.DMA((NSEM,)),
        ],
        compiler_params=pltpu.CompilerParams(vmem_limit_bytes=120 * 1024 * 1024),
    )(
        A_x.reshape(S, D), A_k_cache.reshape(HKV, SK, DH), A_v_cache.reshape(HKV, SK, DH),
        A_wq, A_wo, B_w_r, B_w_gate, B_w_up, B_w_down, c, w_mod,
    )
    return out.reshape(1, S, D)
```

```python
import jax
import jax.numpy as jnp
from jax import lax
import jax.experimental.pallas as pl
import jax.experimental.pallas.tpu as pltpu

S, D, HQ, HKV, DH, SK, W, F = 2048, 1024, 32, 4, 128, 2048, 512, 3584
REP = HQ // HKV
GW = REP * DH
TM = 512
NB = S // TM
QR = TM // HKV
HM = TM // 2
HK = D // 2
WPARTS = 4 * D // DH // HKV
SIDE_STRIDE = 7
SIDE_DIST = 6
PREP_UNROLL = 1
CR = 32
SR = 16
NSL = HM // HKV // SR
FENCE = True
ANCHOR_O = True
LOG2E = 1.4426950408889634
QSCALE = (DH ** -0.5) * LOG2E
EPS = 1e-5
f32, bf16, u32, i32 = jnp.float32, jnp.bfloat16, jnp.uint32, jnp.int32

S_C, S_WMS, S_WMC, S_X0, S_X2, S_WR, S_FIN = range(7)
S_WQ = 7
S_WO = S_WQ + 2 * HKV
S_K = S_WO + HKV
S_V = S_K + HKV
S_X1 = S_V + HKV
S_WMB = S_X1 + 2 * HKV
S_OUT = S_WMB + HKV
NFP = 7
FP = F // NFP
S_WG = S_OUT + NB
S_WU = S_WG + NFP
S_WD = S_WU + NFP
NSEM = S_WD + NFP


def _ln(x):
    m = jnp.mean(x, axis=-1, keepdims=True)
    xc = x - m
    v = jnp.mean(xc * xc, axis=-1, keepdims=True)
    return xc * lax.rsqrt(v + EPS)


def _packs(y):
    r, c = y.shape
    y4 = y.reshape(r // 16, 2, 8, c)
    return pltpu.pack_elementwise([y4[:, 0].reshape(r // 2, c), y4[:, 1].reshape(r // 2, c)], packed_dtype=bf16)


def _halves(w):
    return tuple(pltpu.unpack_elementwise(w, index=n, packed_dtype=bf16, unpacked_dtype=f32) for n in range(2))


def _unpacks(w):
    r, c = w.shape
    lo, hi = (t.reshape(r // 8, 8, c) for t in _halves(w))
    return jnp.stack([lo, hi], axis=1).reshape(2 * r, c)


def _bf(x):
    return pltpu.bitcast(x, bf16)


def _mo(x, m):
    return x if isinstance(x, int) else pl.multiple_of(x, m)


def _recip(l):
    r = pl.reciprocal(l, approx=True)
    return r * (2.0 - l * r)


def _kernel(x_hbm, k_hbm, v_hbm, wq_hbm, wo_hbm, wr_hbm, wg_hbm, wu_hbm, wd_hbm, c_hbm, wm_hbm,
            out_hbm,
            x_v, k_v, v_v, wq_v, wo_v, wr_v, wg_v, wu_v, wd_v, c_v, wm_v,
            h_v, h7_v, o_v, o7_v, o7a_v, q_v, qp_v, ost_v, bq_v, bo_v, acc_v, out_v, x1_v, mod_v, best_v, besti_v, zero_v, zs_ref, sems):
    def cp(src, dst, i):
        return pltpu.make_async_copy(src, dst.bitcast(bf16), sems.at[i])

    def cp_rows(hbm, vm, r0, n, i):
        return cp(hbm.at[pl.ds(_mo(r0, n), n), :], vm.at[pl.ds(_mo(r0 // 2, n // 2), n // 2), :], i)

    def cp_cols(hbm, vm, c0, n, i):
        return cp(hbm.at[:, pl.ds(_mo(c0, 128), n)], vm.at[:, pl.ds(_mo(c0, 128), n)], i)

    def cp_wq(g, half):
        return cp_cols(wq_hbm, wq_v, g * GW + half * (GW // 2), GW // 2, S_WQ + 2 * g + half)

    def cp_k(g):
        return cp(k_hbm.at[g, pl.ds(SK - W, W), :], k_v.at[g], S_K + g)

    def cp_v(g):
        return cp(v_hbm.at[g, pl.ds(SK - W, W), :], v_v.at[g], S_V + g)

    def cp_x1(g, half):
        n = HM // HKV
        return cp_rows(x_hbm, x_v, TM + half * HM + g * n, n, S_X1 + 2 * g + half)


    def cp_wo(g):
        return cp_rows(wo_hbm, wo_v, g * GW, GW, S_WO + g)

    def cp_out(i):
        r0 = i * TM
        return pltpu.make_async_copy(out_v.at[pl.ds(_mo(r0 // 2, TM // 2), TM // 2), :].bitcast(bf16),
                                     out_hbm.at[pl.ds(_mo(r0, TM), TM), :], sems.at[S_OUT + i])

    cp_c = pltpu.make_async_copy(c_hbm, c_v, sems.at[S_C])
    cp_wr = pltpu.make_async_copy(wr_hbm, wr_v, sems.at[S_WR])
    cp_wms = cp_cols(wm_hbm, wm_v, 0, D, S_WMS)
    cp_wmc = cp_cols(wm_hbm, wm_v, D, D, S_WMC)
    cp_x0 = cp_rows(x_hbm, x_v, 0, TM, S_X0)
    cp_x2 = cp_rows(x_hbm, x_v, 2 * TM, S - 2 * TM, S_X2)

    def cp_wmb(n):
        return cp_cols(wm_hbm, wm_v, (2 + n) * D, D, S_WMB + n)

    def cp_ffn(n):
        return (cp_cols(wg_hbm, wg_v, n * FP, FP, S_WG + n), cp_cols(wu_hbm, wu_v, n * FP, FP, S_WU + n),
                cp_rows(wd_hbm, wd_v, n * FP, FP, S_WD + n))

    def group_set(g):
        return (cp_wq(g, 0), cp_x1(g, 0), cp_x1(g, 1), cp_wq(g, 1), cp_k(g), cp_v(g), cp_wo(g))


    for d in (cp_c, cp_x0, cp_wms, cp_wmc) + group_set(0):
        d.start()
    best_v[...] = jnp.full(best_v.shape, -jnp.inf, f32)
    besti_v[...] = jnp.zeros(besti_v.shape, i32)
    zero_v[...] = jnp.zeros(zero_v.shape, u32)
    mod_v[...] = jnp.zeros(mod_v.shape, f32)
    q_v[0:8, 0:128] = jnp.zeros((8, 128), u32)
    qp_v[0:8, 0:128] = jnp.zeros((8, 128), f32)
    for n in range(8):
        zs_ref[n] = 0
    cp_c.wait()
    cc = c_v[...].astype(f32)
    sc = jnp.broadcast_to((cc * jax.nn.sigmoid(cc)).astype(bf16), (16, D))
    cp_x0.wait()
    acc_v[1] = _ln(_bf(x_v[0:TM // 2, :]).astype(f32))
    cp_wms.wait()
    mod_v[:, 0:D] = jnp.dot(sc, _bf(wm_v[:, 0:D]), preferred_element_type=f32)[0:8]
    cp_wmc.wait()
    mod_v[:, D:2 * D] = jnp.dot(sc, _bf(wm_v[:, D:2 * D]), preferred_element_type=f32)[0:8]
    h_v[...] = _packs(acc_v[1] * (1.0 + mod_v[0:1, D:2 * D]) + mod_v[0:1, 0:D])

    def ln1_slice(row0, slot, dst0, normed=False, gate=None):
        sa = mod_v[0:1, 0 * D:1 * D]
        ca1 = 1.0 + mod_v[0:1, 1 * D:2 * D]
        if normed:
            xt, xb = acc_v[1, row0:row0 + 16, :], acc_v[1, row0 + HM:row0 + HM + 16, :]
            norm = lambda t: t
        else:
            xt, xb = (_bf(x_v[pl.ds(_mo(r // 2, 8), 8), :] | gate).astype(f32) for r in (row0, row0 + HM))
            norm = _ln
        dst = pl.ds(_mo(dst0 // 2, 8), 8)
        hs_ = []
        for r in (0, 8):
            top = norm(xt[r:r + 8]) * ca1 + sa
            bot = norm(xb[r:r + 8]) * ca1 + sa
            a11, a12, a21, a22 = top[:, :HK], top[:, HK:], bot[:, :HK], bot[:, HK:]
            hs_.append((a11 + a22, a21 + a22, a11, a22, a11 + a12, a21 - a11, a12 - a22))
        for n in range(7):
            h7_v[slot, n, dst, :] = pltpu.pack_elementwise([hs_[0][n], hs_[1][n]], packed_dtype=bf16)

    def wsum_slice(halves, dst):
        nr = dst.shape[1]
        for rr in range(0, nr, 8):
            for c in range(0, HK, 128):
                b11, b12, b21, b22 = (_halves(halves[kh][rr:rr + 8, nh * HK + c:nh * HK + c + 128])
                                      for kh in range(2) for nh in range(2))
                for n, (p, q, sign) in enumerate(((b11, b22, 1), (b12, b22, -1), (b21, b11, -1),
                                                  (b11, b12, 1), (b21, b22, 1))):
                    dst[n, rr:rr + 8, c:c + 128] = pltpu.pack_elementwise(
                        [u + w if sign > 0 else u - w for u, w in zip(p, q)], packed_dtype=bf16)

    def epi_rows16(src0, row0, slot, acc0, pos0, valid, gate):
        ga = mod_v[0:1, 2 * D:3 * D]
        sb = mod_v[0:1, 3 * D:4 * D]
        cb1 = 1.0 + mod_v[0:1, 4 * D:5 * D]
        gb = mod_v[0:1, 5 * D:6 * D]
        wr = wr_v[...].astype(f32).reshape(1, D)
        rows = pl.ds(_mo(row0 // 2, 8), 8)
        xw = x_v[pl.ds(_mo(src0 // 2, 8), 8), :]
        xs = _halves(xw if isinstance(gate, int) else xw | gate)
        x1s, outs = [], []
        for n in range(2):
            x1 = xs[n] + ga * acc_v[slot, pl.ds(_mo(acc0 + 8 * n, 8), 8), :]
            h2 = _ln(x1) * cb1 + sb
            x1s.append(x1)
            outs.append(x1 + gb * h2)
            r = jnp.broadcast_to(jnp.sum(h2 * wr, axis=-1, keepdims=True), (8, 128))
            ib = row0 + n + 2 * lax.broadcasted_iota(i32, (8, 128), 0)
            sl = pl.ds(pos0 + 8 * n, 8)
            better = r > best_v[sl, :]
            if valid is not True:
                better = better & valid
            best_v[sl, :] = jnp.where(better, r, best_v[sl, :])
            besti_v[sl, :] = jnp.where(better, ib, besti_v[sl, :])
        x1_v[rows, :] = pltpu.pack_elementwise(x1s, packed_dtype=bf16)
        out_v[rows, :] = pltpu.pack_elementwise(outs, packed_dtype=bf16)

    def wq_quad(g):
        def quad(kh, nh, r0=0, nr=HK // 2, c=0, nc=HK):
            return wq_v[pl.ds(_mo(kh * (HK // 2) + r0, 8), nr), pl.ds(_mo(g * GW + nh * HK + c, DH), nc)]
        return quad

    def wo_quad(g):
        def quad(kh, nh, r0=0, nr=HK // 2, c=0, nc=HK):
            return wo_v[pl.ds(_mo((g * GW + kh * HK) // 2 + r0, 8), nr), pl.ds(_mo(nh * HK + c, DH), nc)]
        return quad

    def b_operand(quad, sums, g, n, j):
        if n == 1:
            return quad(0, 0, c=j * DH, nc=DH)
        if n == 4:
            return quad(1, 1, c=j * DH, nc=DH)
        return sums[g, (0, None, 1, 2, None, 3, 4)[n], :, j * DH:(j + 1) * DH]

    def prep_part(g, part):
        nr = HK // 2 // WPARTS
        r0 = part * nr
        rows = pl.ds(_mo(r0, nr), nr)
        wsum_slice([wq_v.at[pl.ds(_mo(kh * (HK // 2) + r0, nr), nr), pl.ds(_mo(g * GW, GW), GW)]
                    for kh in range(2)], bq_v.at[g, :, rows, :])
        wsum_slice([wo_v.at[pl.ds(_mo((g * GW + kh * HK) // 2 + r0, nr), nr), :]
                    for kh in range(2)], bo_v.at[g, :, rows, :])

    def prep(g):
        lax.fori_loop(0, WPARTS, lambda part, _: prep_part(g, part), None)

    def period(i, g, mode):
        hs = i % 2
        if mode == 2:
            @pl.when(i == 0)
            def _():
                @pl.when(g < HKV - 1)
                def _():
                    for d in group_set(g + 1):
                        d.start()

                @pl.when(g == HKV - 1)
                def _():
                    cp_wr.start()
                    cp_x2.start()
                cp_wmb(g).start()
                for d in group_set(g):
                    d.wait()
                prep(g)

            @pl.when((i == 1) & (g == 0))
            def _():
                for n in range(HKV):
                    cp_wmb(n).wait()
                cp_wr.wait()
                cp_x2.wait()
                for part in range(WPARTS):
                    mc = slice(2 * D + part * (4 * D // WPARTS), 2 * D + (part + 1) * (4 * D // WPARTS))
                    mod_v[:, mc] = jnp.dot(sc, _bf(wm_v[:, mc]), preferred_element_type=f32)[0:8]
                    prep_part(0, part)

            @pl.when((g == 0) & (i >= 2))
            def _():
                cp_out(i - 2).start()

            piece = i * HKV + g - HKV

            @pl.when((piece >= 0) & (piece < NFP))
            def _():
                for d in cp_ffn(piece):
                    d.start()

        zero = zero_v[...]
        zz = [zs_ref[n] for n in range(8)]
        zs = zz[0]

        def ln_work(sub, dz):
            if mode == 0 and sub == 0:
                cp_x1(0, 0).wait()
                cp_x1(0, 1).wait()
            q0 = g * (HM // HKV) + sub * SR
            ln1_slice(jnp.minimum(i + 1, NB - 1) * TM + q0, 1 - hs, q0, gate=dz)
            return h7_v[1 - hs, 0, pl.ds(pl.multiple_of(q0 // 2 + zs, 8), 8), 0:128]

        def epi_work(sub, dz):
            toks = None
            for half in range(2):
                q0 = half * HM + g * (HM // HKV) + sub * SR
                src0 = jnp.maximum(i - 1, 0) * TM + q0
                row0 = jnp.where(i == 0, S, (i - 1) * TM) + q0
                pos = (2 * sub + half) * SR
                epi_rows16(src0, row0, 1 - hs, q0, pos, i > 0, dz)
                opq = pl.ds(pl.multiple_of(row0 // 2 + zs, 8), 8)
                ob = pl.ds(pl.multiple_of(pos + zs, 8), 8)
                t = (out_v[opq, 0:128] | x1_v[opq, 0:128]
                     | pltpu.bitcast(best_v[ob, :], u32) | pltpu.bitcast(besti_v[ob, :], u32))
                toks = t if toks is None else toks | t
            return toks

        early, late = [], []
        if mode == 2:
            for sub in range(NSL):
                early += [lambda dz, sub=sub: epi_work(sub, dz)] + [None] * (SIDE_STRIDE - 1)
                late += [lambda dz, sub=sub: ln_work(sub, dz)] + [None] * (SIDE_STRIDE - 1)
        else:
            def h7_first(n):
                ln1_slice(n * SR, 0, n * SR, normed=True)
                return h7_v[0, 0, pl.ds(pl.multiple_of(n * (SR // 2) + zs, 8), 8), 0:128]
            for sub in range(NSL):
                early.append(lambda dz, sub=sub: ln_work(sub, dz))
            for n in range(HM // SR):
                early.append(lambda dz, n=n: h7_first(n))
        pending = [None] * (SIDE_DIST if mode == 2 else 2)

        def anchored(w, extra=None):
            tok = pending.pop(0) if pending else None
            if extra is not None:
                tok = extra if tok is None else tok | extra
            if tok is not None:
                w = jnp.concatenate([w[0:8, :] | jnp.tile(tok & zero, (1, w.shape[1] // 128)), w[8:, :]], axis=0)
            return _bf(w)

        def after(res, queue):
            work = queue.pop(0) if queue else None
            if work is not None:
                src = (qp_v.at[:, 0:128] if queue is early else acc_v.at[hs, :, 0:128]) if mode == 2 else q_v.at[:, 0:128]
                gate = pltpu.bitcast(src[pl.ds(pl.multiple_of(zs, 8), 8), :], u32) & zero
                pending.append(work(jnp.tile(gate, (1, D // 128))))
            else:
                pending.append(None)

        def mm(a, w, queue, extra=None):
            res = jnp.dot(a, anchored(w, extra), preferred_element_type=f32)
            after(res, queue)
            return res

        if mode == 0:
            for hh in range(REP):
                if hh % (REP // 2) == 0:
                    cp_wq(0, hh // (REP // 2)).wait()
                h = _bf(h_v[pl.ds(pl.multiple_of(zz[hh], 8), TM // 2), :])
                qh = mm(h, wq_v[:, pl.ds(_mo(g * GW + hh * DH, DH), DH)], early)
                q_v[:, hh * DH:(hh + 1) * DH] = _packs(qh * QSCALE)
        else:
            quad = wq_quad(g)
            for j in range(HK // DH):
                def d(n):
                    return mm(_bf(h7_v[hs + zz[j], n]), b_operand(quad, bq_v, g, n, j), early)
                L, R = pl.ds(0, DH), pl.ds(DH, DH)
                QL, QR_ = pl.ds(j * DH, DH), pl.ds(HK + j * DH, DH)
                def comb(m, *ops):
                    for r in range(0, HM, CR):
                        mc = m[r:r + CR]
                        for (row, col, kind, qsrc) in ops:
                            rows = pl.ds(row + r, CR)
                            if kind == "set":
                                qp_v[rows, col] = mc
                            elif kind == "add":
                                qp_v[rows, col] += mc
                            elif kind == "sub":
                                qp_v[rows, col] -= mc
                            else:
                                q_v[pl.ds((row + r) // 2, CR // 2), qsrc] = _packs((qp_v[rows, col] + mc) * QSCALE)
                comb(d(0), (0, L, "set", None), (HM, R, "set", None))
                comb(d(1), (HM, R, "sub", None), (HM, L, "set", None))
                comb(d(2), (HM, R, "add", None), (0, R, "set", None))
                comb(d(3), (0, L, "add", None), (HM, L, "q", QL))
                comb(d(4), (0, L, "sub", None), (0, R, "q", QR_))
                comb(d(5), (HM, R, "q", QR_))
                comb(d(6), (0, L, "q", QL))

        if mode == 0:
            cp_k(0).wait()
            cp_v(0).wait()
            for d in group_set(1) + (cp_wmb(0),):
                d.start()
        otok = None
        for hh in range(REP):
            s = lax.dot_general(_bf(q_v[:, hh * DH:(hh + 1) * DH]), anchored(k_v[g]), (((1,), (1,)), ((), ())), preferred_element_type=f32)
            after(s, early)
            m = jnp.max(s, axis=-1, keepdims=True)
            p = jnp.exp2(s - m)
            l = jnp.sum(p, axis=-1, keepdims=True)
            o = mm(p.astype(bf16), v_v[g], early, otok) * _recip(l)
            col = slice((hh % 4) * DH, (hh % 4 + 1) * DH)
            if mode != 2:
                o_v[:, hh * DH:(hh + 1) * DH] = _packs(o)
                oref = o_v
            elif hh < 4:
                top, bot = o[:HM], o[HM:]
                ost_v[:, col] = o
                o7a_v[0, :, col] = _packs(top)
                o7a_v[1, :, col] = _packs(bot - top)
                oref = o7a_v.at[1]
            else:
                a12, a22 = o[:HM], o[HM:]
                a11, a21 = ost_v[0:HM, col], ost_v[HM:TM, col]
                o7_v[0, :, col] = _packs(a11 + a22)
                o7_v[1, :, col] = _packs(a21 + a22)
                o7_v[2, :, col] = _packs(a22)
                o7_v[3, :, col] = _packs(a11 + a12)
                o7_v[4, :, col] = _packs(a12 - a22)
                oref = o7_v.at[4]
            otok = None
            if hh + 2 < REP:
                cc = (hh * DH if mode != 2 else (hh % 4) * DH)
                otok = oref[pl.ds(pl.multiple_of(zs, 8), 8), pl.ds(pl.multiple_of(cc + zs * 128, DH), DH)]

        if mode == 0:
            cp_wo(0).wait()
        if mode != 2:
            for nt in range(D // DH):
                ob = _bf(o_v[pl.ds(pl.multiple_of(zz[nt], 8), TM // 2), :])
                cols = pl.ds(nt * DH, DH)
                contrib = mm(ob, wo_v[pl.ds(_mo(g * GW // 2, GW // 2), GW // 2), cols], late)
                acc_v[hs, :, cols] = contrib if mode == 0 else acc_v[hs, :, cols] + contrib
        else:
            quad = wo_quad(g)

            def d(n, j):
                if n in (2, 5):
                    lhs = o7a_v[(0 if n == 2 else 1) + zz[j]]
                else:
                    lhs = o7_v[(0, 1, None, 2, 3, None, 4)[n] + zz[j]]
                return mm(_bf(lhs), b_operand(quad, bo_v, g, n, j), late)

            def comb(m, j, *ops):
                for r in range(0, HM, CR):
                    mc = m[r:r + CR]
                    for (row, right, kind) in ops:
                        rows, col = pl.ds(row + r, CR), pl.ds(right * HK + j * DH, DH)
                        if kind == "first":
                            acc_v[hs, rows, col] = jnp.where(g == 0, mc, acc_v[hs, rows, col] + mc)
                        elif kind == "add":
                            acc_v[hs, rows, col] += mc
                        else:
                            acc_v[hs, rows, col] -= mc
            for j in range(HK // DH):
                comb(d(2, j), j, (HM, 1, "first"), (0, 1, "first"))
                comb(d(5, j), j, (HM, 1, "add"))
            for j in range(HK // DH):
                comb(d(0, j), j, (0, 0, "first"), (HM, 1, "add"))
                comb(d(1, j), j, (HM, 1, "sub"), (HM, 0, "first"))
                comb(d(3, j), j, (0, 0, "add"), (HM, 0, "add"))
                comb(d(4, j), j, (0, 0, "sub"), (0, 1, "add"))
                comb(d(6, j), j, (0, 0, "add"))
        assert not any(early) and not any(late)

    with jax.named_scope("p00"):
        period(0, 0, 0)
    with jax.named_scope("loopB"):
        def step_b(t, _):
            period(t // HKV, t % HKV, 2)
        lax.fori_loop(1, NB * HKV, step_b, None)
    cp_out(NB - 2).start()

    with jax.named_scope("tail"):
        ga, sb, cb, gb = (mod_v[0:1, n * D:(n + 1) * D] for n in range(2, 6))
        wr = wr_v[...].astype(f32).reshape(1, D)
        last = pl.ds((NB - 1) * TM // 2, TM // 2)
        x1 = _unpacks(x_v[last, :]) + ga * acc_v[(NB - 1) % 2]
        x1_v[last, :] = _packs(x1)
        h2 = _ln(x1) * (1.0 + cb) + sb
        out_v[last, :] = _packs(x1 + gb * h2)
        cp_out(NB - 1).start()
        r = jnp.broadcast_to(jnp.sum(h2 * wr, axis=-1, keepdims=True), (TM, 128))
        pos = lax.broadcasted_iota(i32, (QR, 128), 0)
        pos = (pos & ~15) + 2 * (pos & 7) + ((pos & 15) >> 3)
        for qd in range(HKV):
            rb = r[qd * QR:(qd + 1) * QR]
            better = rb > best_v[...]
            best_v[...] = jnp.where(better, rb, best_v[...])
            besti_v[...] = jnp.where(better, (NB - 1) * TM + qd * QR + pos, besti_v[...])
        bv = best_v[...]
        mx = jnp.max(bv)
        idx = jnp.min(jnp.where(bv == mx, besti_v[...], S))
        idx = jnp.minimum(idx, S - 1)
        base = pl.multiple_of((idx // 16) * 16, 16)
        pb = pl.ds(pl.multiple_of(base // 2, 8), 8)
        x1 = _bf(x1_v[pb, :]).astype(f32)
        h2 = _ln(x1) * (1.0 + cb) + sb
        hsel = h2.astype(bf16)
        r_sel = jnp.sum(hsel.astype(f32) * wr, axis=-1, keepdims=True)
        for n in range(NFP):
            cp_cols(wg_hbm, wg_v, n * FP, FP, S_WG + n).wait()
        gg = jnp.dot(hsel, _bf(wg_v[...]), preferred_element_type=f32)
        for n in range(NFP):
            cp_cols(wu_hbm, wu_v, n * FP, FP, S_WU + n).wait()
        uu = jnp.dot(hsel, _bf(wu_v[...]), preferred_element_type=f32)
        a = (gg * jax.nn.sigmoid(gg) * uu).astype(bf16)
        for n in range(NFP):
            cp_rows(wd_hbm, wd_v, n * FP, FP, S_WD + n).wait()
        y = jnp.dot(a, _bf(wd_v[...]), preferred_element_type=f32)
        y = y * jax.nn.sigmoid(r_sel)
        rows = base + lax.broadcasted_iota(i32, (16, D), 0)
        new = (x1 + gb * (h2 + y)).astype(bf16)
        for i in range(NB):
            cp_out(i).wait()
        out_v[pb, :] = pltpu.bitcast(jnp.where(rows == idx, new, _bf(out_v[pb, :])), u32)
        fin = pltpu.make_async_copy(out_v.at[pb, :].bitcast(bf16), out_hbm.at[pl.ds(base, 16), :], sems.at[S_FIN])
        fin.start()
        fin.wait()


@jax.jit
def pallas_adaLN_cond__sliding_block_cached__moe_arch_mod__prompt_kernel(
    A_x, A_k_cache, A_v_cache, A_wq, A_wo, B_x, B_w_r, B_w_gate, B_w_up, B_w_down, c, w_mod,
):
    anyspec = pl.BlockSpec(memory_space=pl.ANY)
    out = pl.pallas_call(
        _kernel,
        out_shape=jax.ShapeDtypeStruct((S, D), bf16),
        in_specs=[anyspec] * 11,
        out_specs=anyspec,
        scratch_shapes=[
            pltpu.VMEM((S // 2, D), u32),
            pltpu.VMEM((HKV, W // 2, DH), u32),
            pltpu.VMEM((HKV, W // 2, DH), u32),
            pltpu.VMEM((D // 2, HQ * DH), u32),
            pltpu.VMEM((HQ * DH // 2, D), u32),
            pltpu.VMEM((D,), bf16),
            pltpu.VMEM((D // 2, F), u32),
            pltpu.VMEM((D // 2, F), u32),
            pltpu.VMEM((F // 2, D), u32),
            pltpu.VMEM((1, D), bf16),
            pltpu.VMEM((D // 2, 6 * D), u32),
            pltpu.VMEM((TM // 2, D), u32),
            pltpu.VMEM((2, 7, HM // 2, HK), u32),
            pltpu.VMEM((TM // 2, GW), u32),
            pltpu.VMEM((5, HM // 2, HK), u32),
            pltpu.VMEM((2, HM // 2, HK), u32),
            pltpu.VMEM((TM // 2, GW), u32),
            pltpu.VMEM((TM, 2 * DH), f32),
            pltpu.VMEM((TM, HK), f32),
            pltpu.VMEM((HKV, 5, HK // 2, HK), u32),
            pltpu.VMEM((HKV, 5, HK // 2, HK), u32),
            pltpu.VMEM((2, TM, D), f32),
            pltpu.VMEM((S // 2 + TM // 2, D), u32),
            pltpu.VMEM((S // 2 + TM // 2, D), u32),
            pltpu.VMEM((8, 6 * D), f32),
            pltpu.VMEM((QR, 128), f32),
            pltpu.VMEM((QR, 128), i32),
            pltpu.VMEM((8, 128), u32),
            pltpu.SMEM((8,), i32),
            pltpu.SemaphoreType.DMA((NSEM,)),
        ],
        compiler_params=pltpu.CompilerParams(vmem_limit_bytes=120 * 1024 * 1024),
    )(
        A_x.reshape(S, D), A_k_cache.reshape(HKV, SK, DH), A_v_cache.reshape(HKV, SK, DH),
        A_wq, A_wo, B_w_r, B_w_gate, B_w_up, B_w_down, c, w_mod,
    )
    return out.reshape(1, S, D)
```

```python
import jax
import jax.numpy as jnp
from jax import lax
import jax.experimental.pallas as pl
import jax.experimental.pallas.tpu as pltpu

S, D, HQ, HKV, DH, SK, W, F = 2048, 1024, 32, 4, 128, 2048, 512, 3584
REP = HQ // HKV
GW = REP * DH
TM = 512
NB = S // TM
QR = TM // HKV
HM = TM // 2
HK = D // 2
WPARTS = 8
SIDE_STRIDE = 7
SIDE_DIST = 4
CR = 32
SR = 16
NSL = HM // HKV // SR
LOG2E = 1.4426950408889634
QSCALE = (DH ** -0.5) * LOG2E
EPS = 1e-5
f32, bf16, u32, i32 = jnp.float32, jnp.bfloat16, jnp.uint32, jnp.int32

S_C, S_WMS, S_WMC, S_X0, S_X2, S_WR, S_FIN, S_WQ0 = range(8)
S_WQ = 8
S_WO = S_WQ + 2 * HKV
S_K = S_WO + HKV
S_V = S_K + HKV
S_X1 = S_V + HKV
S_WMB = S_X1 + 2 * HKV
S_OUT = S_WMB + HKV
NFP = 7
FP = F // NFP
S_WG = S_OUT + NB
S_WU = S_WG + NFP
S_WD = S_WU + NFP
NSEM = S_WD + NFP


def _ln(x):
    m = jnp.mean(x, axis=-1, keepdims=True)
    xc = x - m
    v = jnp.mean(xc * xc, axis=-1, keepdims=True)
    return xc * lax.rsqrt(v + EPS)


def _packs(y):
    r, c = y.shape
    y4 = y.reshape(r // 16, 2, 8, c)
    return pltpu.pack_elementwise([y4[:, 0].reshape(r // 2, c), y4[:, 1].reshape(r // 2, c)], packed_dtype=bf16)


def _halves(w):
    return tuple(pltpu.unpack_elementwise(w, index=n, packed_dtype=bf16, unpacked_dtype=f32) for n in range(2))


def _unpacks(w):
    r, c = w.shape
    lo, hi = (t.reshape(r // 8, 8, c) for t in _halves(w))
    return jnp.stack([lo, hi], axis=1).reshape(2 * r, c)


def _bf(x):
    return pltpu.bitcast(x, bf16)


def _mo(x, m):
    return x if isinstance(x, int) else pl.multiple_of(x, m)


def _recip(l):
    r = pl.reciprocal(l, approx=True)
    return r * (2.0 - l * r)


def _kernel(x_hbm, k_hbm, v_hbm, wq_hbm, wo_hbm, wr_hbm, wg_hbm, wu_hbm, wd_hbm, c_hbm, wm_hbm,
            out_hbm,
            x_v, k_v, v_v, wq_v, wo_v, wr_v, wg_v, wu_v, wd_v, c_v, wm_v,
            h_v, h7_v, o_v, o7_v, o7a_v, q_v, qp_v, ost_v, bq_v, bo_v, acc_v, out_v, x1_v, mod_v, best_v, besti_v, zero_v, zs_ref, sems):
    def cp(src, dst, i):
        return pltpu.make_async_copy(src, dst.bitcast(bf16), sems.at[i])

    def cp_rows(hbm, vm, r0, n, i):
        return cp(hbm.at[pl.ds(_mo(r0, n), n), :], vm.at[pl.ds(_mo(r0 // 2, n // 2), n // 2), :], i)

    def cp_cols(hbm, vm, c0, n, i):
        return cp(hbm.at[:, pl.ds(_mo(c0, 128), n)], vm.at[:, pl.ds(_mo(c0, 128), n)], i)

    def cp_wq(g, half):
        return cp_cols(wq_hbm, wq_v, g * GW + half * (GW // 2), GW // 2, S_WQ + 2 * g + half)

    def cp_k(g):
        return cp(k_hbm.at[g, pl.ds(SK - W, W), :], k_v.at[g], S_K + g)

    def cp_v(g):
        return cp(v_hbm.at[g, pl.ds(SK - W, W), :], v_v.at[g], S_V + g)

    def cp_x1(g, half):
        n = HM // HKV
        return cp_rows(x_hbm, x_v, TM + half * HM + g * n, n, S_X1 + 2 * g + half)


    def cp_wo(g):
        return cp_rows(wo_hbm, wo_v, g * GW, GW, S_WO + g)

    def cp_out(i):
        r0 = i * TM
        return pltpu.make_async_copy(out_v.at[pl.ds(_mo(r0 // 2, TM // 2), TM // 2), :].bitcast(bf16),
                                     out_hbm.at[pl.ds(_mo(r0, TM), TM), :], sems.at[S_OUT + i])

    cp_c = pltpu.make_async_copy(c_hbm, c_v, sems.at[S_C])
    cp_wr = pltpu.make_async_copy(wr_hbm, wr_v, sems.at[S_WR])
    cp_wms = cp_cols(wm_hbm, wm_v, 0, D, S_WMS)
    cp_wmc = cp_cols(wm_hbm, wm_v, D, D, S_WMC)
    cp_x0 = cp_rows(x_hbm, x_v, 0, TM, S_X0)
    cp_x2 = cp_rows(x_hbm, x_v, 2 * TM, S - 2 * TM, S_X2)

    def cp_wmb(n):
        return cp_cols(wm_hbm, wm_v, (2 + n) * D, D, S_WMB + n)

    def cp_ffn(n):
        return (cp_cols(wg_hbm, wg_v, n * FP, FP, S_WG + n), cp_cols(wu_hbm, wu_v, n * FP, FP, S_WU + n),
                cp_rows(wd_hbm, wd_v, n * FP, FP, S_WD + n))

    def group_set(g):
        return (cp_wq(g, 0), cp_x1(g, 0), cp_x1(g, 1), cp_wq(g, 1), cp_k(g), cp_v(g), cp_wo(g))


    cp_wq00 = cp_cols(wq_hbm, wq_v, 0, DH, S_WQ0)
    cp_wq01 = cp_cols(wq_hbm, wq_v, DH, GW // 2 - DH, S_WQ)
    for d in (cp_c, cp_wr, cp_x0, cp_wms, cp_wmc, cp_wq00, cp_wq01, cp_x1(0, 0), cp_x1(0, 1), cp_wq(0, 1),
              cp_k(0), cp_v(0), cp_wo(0)):
        d.start()
    best_v[...] = jnp.full(best_v.shape, -jnp.inf, f32)
    besti_v[...] = jnp.zeros(besti_v.shape, i32)
    zero_v[...] = jnp.zeros(zero_v.shape, u32)
    mod_v[...] = jnp.zeros(mod_v.shape, f32)
    q_v[0:8, 0:128] = jnp.zeros((8, 128), u32)
    qp_v[0:8, 0:128] = jnp.zeros((8, 128), f32)
    for n in range(8):
        zs_ref[n] = 0
    cp_c.wait()
    cp_wr.wait()
    cc = c_v[...].astype(f32)
    sc = jnp.broadcast_to((cc * jax.nn.sigmoid(cc)).astype(bf16), (16, D))
    cp_x0.wait()
    acc_v[1] = _ln(_bf(x_v[0:TM // 2, :]).astype(f32))
    cp_wms.wait()
    mod_v[:, 0:D] = jnp.dot(sc, _bf(wm_v[:, 0:D]), preferred_element_type=f32)[0:8]
    cp_wmc.wait()
    mod_v[:, D:2 * D] = jnp.dot(sc, _bf(wm_v[:, D:2 * D]), preferred_element_type=f32)[0:8]
    h_v[...] = _packs(acc_v[1] * (1.0 + mod_v[0:1, D:2 * D]) + mod_v[0:1, 0:D])

    def ln1_slice(row0, slot, dst0, normed=False, gate=None):
        sa = mod_v[0:1, 0 * D:1 * D]
        ca1 = 1.0 + mod_v[0:1, 1 * D:2 * D]
        if normed:
            xt, xb = acc_v[1, row0:row0 + 16, :], acc_v[1, row0 + HM:row0 + HM + 16, :]
            norm = lambda t: t
        else:
            xt, xb = (_bf(x_v[pl.ds(_mo(r // 2, 8), 8), :] | gate).astype(f32) for r in (row0, row0 + HM))
            norm = _ln
        dst = pl.ds(_mo(dst0 // 2, 8), 8)
        hs_ = []
        for r in (0, 8):
            top = norm(xt[r:r + 8]) * ca1 + sa
            bot = norm(xb[r:r + 8]) * ca1 + sa
            a11, a12, a21, a22 = top[:, :HK], top[:, HK:], bot[:, :HK], bot[:, HK:]
            hs_.append((a11 + a22, a21 + a22, a11, a22, a11 + a12, a21 - a11, a12 - a22))
        for n in range(7):
            h7_v[slot, n, dst, :] = pltpu.pack_elementwise([hs_[0][n], hs_[1][n]], packed_dtype=bf16)

    def wsum_slice(halves, dst):
        nr = dst.shape[1]
        for rr in range(0, nr, 8):
            for c in range(0, HK, 128):
                b11, b12, b21, b22 = (_halves(halves[kh][rr:rr + 8, nh * HK + c:nh * HK + c + 128])
                                      for kh in range(2) for nh in range(2))
                for n, (p, q, sign) in enumerate(((b11, b22, 1), (b12, b22, -1), (b21, b11, -1),
                                                  (b11, b12, 1), (b21, b22, 1))):
                    dst[n, rr:rr + 8, c:c + 128] = pltpu.pack_elementwise(
                        [u + w if sign > 0 else u - w for u, w in zip(p, q)], packed_dtype=bf16)

    def epi_rows16(src0, row0, slot, acc0, pos0, valid, gate):
        ga = mod_v[0:1, 2 * D:3 * D]
        sb = mod_v[0:1, 3 * D:4 * D]
        cb1 = 1.0 + mod_v[0:1, 4 * D:5 * D]
        gb = mod_v[0:1, 5 * D:6 * D]
        wr = wr_v[...].astype(f32).reshape(1, D)
        rows = pl.ds(_mo(row0 // 2, 8), 8)
        xw = x_v[pl.ds(_mo(src0 // 2, 8), 8), :]
        xs = _halves(xw if isinstance(gate, int) else xw | gate)
        x1s, outs = [], []
        for n in range(2):
            x1 = xs[n] + ga * acc_v[slot, pl.ds(_mo(acc0 + 8 * n, 8), 8), :]
            h2 = _ln(x1) * cb1 + sb
            x1s.append(x1)
            outs.append(x1 + gb * h2)
            r = jnp.broadcast_to(jnp.sum(h2 * wr, axis=-1, keepdims=True), (8, 128))
            ib = row0 + n + 2 * lax.broadcasted_iota(i32, (8, 128), 0)
            sl = pl.ds(pos0 + 8 * n, 8)
            better = r > best_v[sl, :]
            if valid is not True:
                better = better & valid
            best_v[sl, :] = jnp.where(better, r, best_v[sl, :])
            besti_v[sl, :] = jnp.where(better, ib, besti_v[sl, :])
        x1_v[rows, :] = pltpu.pack_elementwise(x1s, packed_dtype=bf16)
        out_v[rows, :] = pltpu.pack_elementwise(outs, packed_dtype=bf16)

    def wq_quad(g):
        def quad(kh, nh, r0=0, nr=HK // 2, c=0, nc=HK):
            return wq_v[pl.ds(_mo(kh * (HK // 2) + r0, 8), nr), pl.ds(_mo(g * GW + nh * HK + c, DH), nc)]
        return quad

    def wo_quad(g):
        def quad(kh, nh, r0=0, nr=HK // 2, c=0, nc=HK):
            return wo_v[pl.ds(_mo((g * GW + kh * HK) // 2 + r0, 8), nr), pl.ds(_mo(nh * HK + c, DH), nc)]
        return quad

    def b_operand(quad, sums, g, n, j):
        if n == 1:
            return quad(0, 0, c=j * DH, nc=DH)
        if n == 4:
            return quad(1, 1, c=j * DH, nc=DH)
        return sums[g, (0, None, 1, 2, None, 3, 4)[n], :, j * DH:(j + 1) * DH]

    def prep_part(g, part):
        nr = HK // 2 // WPARTS
        r0 = part * nr
        rows = pl.ds(_mo(r0, nr), nr)
        wsum_slice([wq_v.at[pl.ds(_mo(kh * (HK // 2) + r0, nr), nr), pl.ds(_mo(g * GW, GW), GW)]
                    for kh in range(2)], bq_v.at[g, :, rows, :])
        wsum_slice([wo_v.at[pl.ds(_mo((g * GW + kh * HK) // 2 + r0, nr), nr), :]
                    for kh in range(2)], bo_v.at[g, :, rows, :])

    def prep(g):
        lax.fori_loop(0, WPARTS, lambda part, _: prep_part(g, part), None)

    def period(i, g, mode):
        hs = i % 2
        if mode == 2:
            @pl.when(i == 0)
            def _():
                @pl.when(g < HKV - 1)
                def _():
                    for d in group_set(g + 1):
                        d.start()

                @pl.when(g == HKV - 1)
                def _():
                    cp_x2.start()
                cp_wmb(g).start()
                for d in group_set(g):
                    d.wait()
                prep(g)

            @pl.when((i == 1) & (g == 0))
            def _():
                for n in range(HKV):
                    cp_wmb(n).wait()
                cp_x2.wait()
                for part in range(WPARTS):
                    mc = slice(2 * D + part * (4 * D // WPARTS), 2 * D + (part + 1) * (4 * D // WPARTS))
                    mod_v[:, mc] = jnp.dot(sc, _bf(wm_v[:, mc]), preferred_element_type=f32)[0:8]
                    prep_part(0, part)

            @pl.when((g == 0) & (i >= 2))
            def _():
                cp_out(i - 2).start()

            piece = i * HKV + g - HKV

            @pl.when((piece >= 0) & (piece < NFP))
            def _():
                for d in cp_ffn(piece):
                    d.start()

        zero = zero_v[...]
        zz = [zs_ref[n] for n in range(8)]
        zs = zz[0]

        def ln_work(sub, dz):
            if mode == 0 and sub == 0:
                cp_x1(0, 0).wait()
                cp_x1(0, 1).wait()
            q0 = g * (HM // HKV) + sub * SR
            ln1_slice(jnp.minimum(i + 1, NB - 1) * TM + q0, 1 - hs, q0, gate=dz)
            return h7_v[1 - hs, 0, pl.ds(pl.multiple_of(q0 // 2 + zs, 8), 8), 0:128]

        def epi_work(sub, dz):
            toks = None
            for half in range(2):
                q0 = half * HM + g * (HM // HKV) + sub * SR
                src0 = jnp.maximum(i - 1, 0) * TM + q0
                row0 = jnp.where(i == 0, S, (i - 1) * TM) + q0
                pos = (2 * sub + half) * SR
                epi_rows16(src0, row0, 1 - hs, q0, pos, i > 0, dz)
                opq = pl.ds(pl.multiple_of(row0 // 2 + zs, 8), 8)
                ob = pl.ds(pl.multiple_of(pos + zs, 8), 8)
                t = (out_v[opq, 0:128] | x1_v[opq, 0:128]
                     | pltpu.bitcast(best_v[ob, :], u32) | pltpu.bitcast(besti_v[ob, :], u32))
                toks = t if toks is None else toks | t
            return toks

        early, late = [], []
        if mode == 2:
            for sub in range(NSL):
                early += [lambda dz, sub=sub: epi_work(sub, dz)] + [None] * (SIDE_STRIDE - 1)
                late += [lambda dz, sub=sub: ln_work(sub, dz)] + [None] * (SIDE_STRIDE - 1)
        else:
            def h7_first(n):
                ln1_slice(n * SR, 0, n * SR, normed=True)
                return h7_v[0, 0, pl.ds(pl.multiple_of(n * (SR // 2) + zs, 8), 8), 0:128]
            for sub in range(NSL):
                early.append(lambda dz, sub=sub: ln_work(sub, dz))
            for n in range(HM // SR):
                early.append(lambda dz, n=n: h7_first(n))
        pending = [None] * (SIDE_DIST if mode == 2 else 2)

        def anchored(w, extra=None):
            tok = pending.pop(0) if pending else None
            if extra is not None:
                tok = extra if tok is None else tok | extra
            if tok is not None:
                w = jnp.concatenate([w[0:8, :] | jnp.tile(tok & zero, (1, w.shape[1] // 128)), w[8:, :]], axis=0)
            return _bf(w)

        def after(res, queue):
            work = queue.pop(0) if queue else None
            if work is not None:
                src = (qp_v.at[:, 0:128] if queue is early else acc_v.at[hs, :, 0:128]) if mode == 2 else q_v.at[:, 0:128]
                gate = pltpu.bitcast(src[pl.ds(pl.multiple_of(zs, 8), 8), :], u32) & zero
                pending.append(work(jnp.tile(gate, (1, D // 128))))
            else:
                pending.append(None)

        def mm(a, w, queue, extra=None):
            res = jnp.dot(a, anchored(w, extra), preferred_element_type=f32)
            after(res, queue)
            return res

        if mode == 0:
            for hh in range(REP):
                if hh == 0:
                    cp_wq00.wait()
                elif hh == 1:
                    cp_wq01.wait()
                elif hh == REP // 2:
                    cp_wq(0, 1).wait()
                h = _bf(h_v[pl.ds(pl.multiple_of(zz[hh], 8), TM // 2), :])
                qh = mm(h, wq_v[:, pl.ds(_mo(g * GW + hh * DH, DH), DH)], early)
                q_v[:, hh * DH:(hh + 1) * DH] = _packs(qh * QSCALE)
        else:
            quad = wq_quad(g)
            for j in range(HK // DH):
                def d(n):
                    return mm(_bf(h7_v[hs + zz[j], n]), b_operand(quad, bq_v, g, n, j), early)
                L, R = pl.ds(0, DH), pl.ds(DH, DH)
                QL, QR_ = pl.ds(j * DH, DH), pl.ds(HK + j * DH, DH)
                def comb(m, *ops):
                    for r in range(0, HM, CR):
                        mc = m[r:r + CR]
                        for (row, col, kind, qsrc) in ops:
                            rows = pl.ds(row + r, CR)
                            if kind == "set":
                                qp_v[rows, col] = mc
                            elif kind == "add":
                                qp_v[rows, col] += mc
                            elif kind == "sub":
                                qp_v[rows, col] -= mc
                            else:
                                q_v[pl.ds((row + r) // 2, CR // 2), qsrc] = _packs((qp_v[rows, col] + mc) * QSCALE)
                comb(d(0), (0, L, "set", None), (HM, R, "set", None))
                comb(d(1), (HM, R, "sub", None), (HM, L, "set", None))
                comb(d(2), (HM, R, "add", None), (0, R, "set", None))
                comb(d(3), (0, L, "add", None), (HM, L, "q", QL))
                comb(d(4), (0, L, "sub", None), (0, R, "q", QR_))
                comb(d(5), (HM, R, "q", QR_))
                comb(d(6), (0, L, "q", QL))

        if mode == 0:
            cp_k(0).wait()
            cp_v(0).wait()
            for d in group_set(1) + (cp_wmb(0),):
                d.start()
        otok = None
        for hh in range(REP):
            s = lax.dot_general(_bf(q_v[:, hh * DH:(hh + 1) * DH]), anchored(k_v[g]), (((1,), (1,)), ((), ())), preferred_element_type=f32)
            after(s, early)
            m = jnp.max(s, axis=-1, keepdims=True)
            p = jnp.exp2(s - m)
            l = jnp.sum(p, axis=-1, keepdims=True)
            o = mm(p.astype(bf16), v_v[g], early, otok) * _recip(l)
            col = slice((hh % 4) * DH, (hh % 4 + 1) * DH)
            if mode != 2:
                o_v[:, hh * DH:(hh + 1) * DH] = _packs(o)
                oref = o_v
            elif hh < 4:
                top, bot = o[:HM], o[HM:]
                ost_v[:, col] = o
                o7a_v[0, :, col] = _packs(top)
                o7a_v[1, :, col] = _packs(bot - top)
                oref = o7a_v.at[1]
            else:
                a12, a22 = o[:HM], o[HM:]
                a11, a21 = ost_v[0:HM, col], ost_v[HM:TM, col]
                o7_v[0, :, col] = _packs(a11 + a22)
                o7_v[1, :, col] = _packs(a21 + a22)
                o7_v[2, :, col] = _packs(a22)
                o7_v[3, :, col] = _packs(a11 + a12)
                o7_v[4, :, col] = _packs(a12 - a22)
                oref = o7_v.at[4]
            otok = None
            if hh + 2 < REP:
                cc = (hh * DH if mode != 2 else (hh % 4) * DH)
                otok = oref[pl.ds(pl.multiple_of(zs, 8), 8), pl.ds(pl.multiple_of(cc + zs * 128, DH), DH)]

        if mode == 0:
            cp_wo(0).wait()
        if mode != 2:
            for nt in range(D // DH):
                ob = _bf(o_v[pl.ds(pl.multiple_of(zz[nt], 8), TM // 2), :])
                cols = pl.ds(nt * DH, DH)
                contrib = mm(ob, wo_v[pl.ds(_mo(g * GW // 2, GW // 2), GW // 2), cols], late)
                acc_v[hs, :, cols] = contrib if mode == 0 else acc_v[hs, :, cols] + contrib
        else:
            quad = wo_quad(g)

            def d(n, j):
                if n in (2, 5):
                    lhs = o7a_v[(0 if n == 2 else 1) + zz[j]]
                else:
                    lhs = o7_v[(0, 1, None, 2, 3, None, 4)[n] + zz[j]]
                return mm(_bf(lhs), b_operand(quad, bo_v, g, n, j), late)

            def comb(m, j, *ops):
                for r in range(0, HM, CR):
                    mc = m[r:r + CR]
                    for (row, right, kind) in ops:
                        rows, col = pl.ds(row + r, CR), pl.ds(right * HK + j * DH, DH)
                        if kind == "first":
                            acc_v[hs, rows, col] = jnp.where(g == 0, mc, acc_v[hs, rows, col] + mc)
                        elif kind == "add":
                            acc_v[hs, rows, col] += mc
                        else:
                            acc_v[hs, rows, col] -= mc
            for j in range(HK // DH):
                comb(d(2, j), j, (HM, 1, "first"), (0, 1, "first"))
                comb(d(5, j), j, (HM, 1, "add"))
            for j in range(HK // DH):
                comb(d(0, j), j, (0, 0, "first"), (HM, 1, "add"))
                comb(d(1, j), j, (HM, 1, "sub"), (HM, 0, "first"))
                comb(d(3, j), j, (0, 0, "add"), (HM, 0, "add"))
                comb(d(4, j), j, (0, 0, "sub"), (0, 1, "add"))
                comb(d(6, j), j, (0, 0, "add"))
        assert not any(early) and not any(late)

    with jax.named_scope("p00"):
        period(0, 0, 0)
    with jax.named_scope("loopB"):
        def step_b(t, _):
            period(t // HKV, t % HKV, 2)
        lax.fori_loop(1, NB * HKV, step_b, None)
    cp_out(NB - 2).start()

    with jax.named_scope("tail"):
        ga, sb, cb, gb = (mod_v[0:1, n * D:(n + 1) * D] for n in range(2, 6))
        wr = wr_v[...].astype(f32).reshape(1, D)
        last = pl.ds((NB - 1) * TM // 2, TM // 2)
        x1 = _unpacks(x_v[last, :]) + ga * acc_v[(NB - 1) % 2]
        x1_v[last, :] = _packs(x1)
        h2 = _ln(x1) * (1.0 + cb) + sb
        out_v[last, :] = _packs(x1 + gb * h2)
        cp_out(NB - 1).start()
        r = jnp.broadcast_to(jnp.sum(h2 * wr, axis=-1, keepdims=True), (TM, 128))
        pos = lax.broadcasted_iota(i32, (QR, 128), 0)
        pos = (pos & ~15) + 2 * (pos & 7) + ((pos & 15) >> 3)
        for qd in range(HKV):
            rb = r[qd * QR:(qd + 1) * QR]
            better = rb > best_v[...]
            best_v[...] = jnp.where(better, rb, best_v[...])
            besti_v[...] = jnp.where(better, (NB - 1) * TM + qd * QR + pos, besti_v[...])
        bv = best_v[...]
        mx = jnp.max(bv)
        idx = jnp.min(jnp.where(bv == mx, besti_v[...], S))
        idx = jnp.minimum(idx, S - 1)
        base = pl.multiple_of((idx // 16) * 16, 16)
        pb = pl.ds(pl.multiple_of(base // 2, 8), 8)
        x1 = _bf(x1_v[pb, :]).astype(f32)
        h2 = _ln(x1) * (1.0 + cb) + sb
        hsel = h2.astype(bf16)
        r_sel = jnp.sum(hsel.astype(f32) * wr, axis=-1, keepdims=True)
        for n in range(NFP):
            cp_cols(wg_hbm, wg_v, n * FP, FP, S_WG + n).wait()
        gg = jnp.dot(hsel, _bf(wg_v[...]), preferred_element_type=f32)
        for n in range(NFP):
            cp_cols(wu_hbm, wu_v, n * FP, FP, S_WU + n).wait()
        uu = jnp.dot(hsel, _bf(wu_v[...]), preferred_element_type=f32)
        a = (gg * jax.nn.sigmoid(gg) * uu).astype(bf16)
        for n in range(NFP):
            cp_rows(wd_hbm, wd_v, n * FP, FP, S_WD + n).wait()
        y = jnp.dot(a, _bf(wd_v[...]), preferred_element_type=f32)
        y = y * jax.nn.sigmoid(r_sel)
        rows = base + lax.broadcasted_iota(i32, (16, D), 0)
        new = (x1 + gb * (h2 + y)).astype(bf16)
        for i in range(NB):
            cp_out(i).wait()
        out_v[pb, :] = pltpu.bitcast(jnp.where(rows == idx, new, _bf(out_v[pb, :])), u32)
        fin = pltpu.make_async_copy(out_v.at[pb, :].bitcast(bf16), out_hbm.at[pl.ds(base, 16), :], sems.at[S_FIN])
        fin.start()
        fin.wait()


@jax.jit
def pallas_adaLN_cond__sliding_block_cached__moe_arch_mod__prompt_kernel(
    A_x, A_k_cache, A_v_cache, A_wq, A_wo, B_x, B_w_r, B_w_gate, B_w_up, B_w_down, c, w_mod,
):
    anyspec = pl.BlockSpec(memory_space=pl.ANY)
    out = pl.pallas_call(
        _kernel,
        out_shape=jax.ShapeDtypeStruct((S, D), bf16),
        in_specs=[anyspec] * 11,
        out_specs=anyspec,
        scratch_shapes=[
            pltpu.VMEM((S // 2, D), u32),
            pltpu.VMEM((HKV, W // 2, DH), u32),
            pltpu.VMEM((HKV, W // 2, DH), u32),
            pltpu.VMEM((D // 2, HQ * DH), u32),
            pltpu.VMEM((HQ * DH // 2, D), u32),
            pltpu.VMEM((D,), bf16),
            pltpu.VMEM((D // 2, F), u32),
            pltpu.VMEM((D // 2, F), u32),
            pltpu.VMEM((F // 2, D), u32),
            pltpu.VMEM((1, D), bf16),
            pltpu.VMEM((D // 2, 6 * D), u32),
            pltpu.VMEM((TM // 2, D), u32),
            pltpu.VMEM((2, 7, HM // 2, HK), u32),
            pltpu.VMEM((TM // 2, GW), u32),
            pltpu.VMEM((5, HM // 2, HK), u32),
            pltpu.VMEM((2, HM // 2, HK), u32),
            pltpu.VMEM((TM // 2, GW), u32),
            pltpu.VMEM((TM, 2 * DH), f32),
            pltpu.VMEM((TM, HK), f32),
            pltpu.VMEM((HKV, 5, HK // 2, HK), u32),
            pltpu.VMEM((HKV, 5, HK // 2, HK), u32),
            pltpu.VMEM((2, TM, D), f32),
            pltpu.VMEM((S // 2 + TM // 2, D), u32),
            pltpu.VMEM((S // 2 + TM // 2, D), u32),
            pltpu.VMEM((8, 6 * D), f32),
            pltpu.VMEM((QR, 128), f32),
            pltpu.VMEM((QR, 128), i32),
            pltpu.VMEM((8, 128), u32),
            pltpu.SMEM((8,), i32),
            pltpu.SemaphoreType.DMA((NSEM,)),
        ],
        compiler_params=pltpu.CompilerParams(vmem_limit_bytes=120 * 1024 * 1024),
    )(
        A_x.reshape(S, D), A_k_cache.reshape(HKV, SK, DH), A_v_cache.reshape(HKV, SK, DH),
        A_wq, A_wo, B_w_r, B_w_gate, B_w_up, B_w_down, c, w_mod,
    )
    return out.reshape(1, S, D)
```

```python
import jax
import jax.numpy as jnp
from jax import lax
import jax.experimental.pallas as pl
import jax.experimental.pallas.tpu as pltpu

S, D, HQ, HKV, DH, SK, W, F = 2048, 1024, 32, 4, 128, 2048, 512, 3584
REP = HQ // HKV
GW = REP * DH
TM = 512
NB = S // TM
QR = TM // HKV
HM = TM // 2
HK = D // 2
WPARTS = 8
SIDE_STRIDE = 7
SIDE_DIST = 4
CR = 32
SR = 16
NSL = HM // HKV // SR
LOG2E = 1.4426950408889634
QSCALE = (DH ** -0.5) * LOG2E
EPS = 1e-5
f32, bf16, u32, i32 = jnp.float32, jnp.bfloat16, jnp.uint32, jnp.int32

S_C, S_WMS, S_WMC, S_X0, S_X2, S_WR, S_FIN, S_WQ0 = range(8)
S_WQ = 8
S_WO = S_WQ + 2 * HKV
S_K = S_WO + HKV
S_V = S_K + HKV
S_X1 = S_V + HKV
S_WMB = S_X1 + 2 * HKV
S_OUT = S_WMB + HKV
NFP = 7
FP = F // NFP
S_WG = S_OUT + NB
S_WU = S_WG + NFP
S_WD = S_WU + NFP
NSEM = S_WD + NFP


def _ln(x):
    m = jnp.mean(x, axis=-1, keepdims=True)
    xc = x - m
    v = jnp.mean(xc * xc, axis=-1, keepdims=True)
    return xc * lax.rsqrt(v + EPS)


def _packs(y):
    r, c = y.shape
    y4 = y.reshape(r // 16, 2, 8, c)
    return pltpu.pack_elementwise([y4[:, 0].reshape(r // 2, c), y4[:, 1].reshape(r // 2, c)], packed_dtype=bf16)


def _halves(w):
    return tuple(pltpu.unpack_elementwise(w, index=n, packed_dtype=bf16, unpacked_dtype=f32) for n in range(2))


def _unpacks(w):
    r, c = w.shape
    lo, hi = (t.reshape(r // 8, 8, c) for t in _halves(w))
    return jnp.stack([lo, hi], axis=1).reshape(2 * r, c)


def _bf(x):
    return pltpu.bitcast(x, bf16)


def _mo(x, m):
    return x if isinstance(x, int) else pl.multiple_of(x, m)


def _recip(l):
    r = pl.reciprocal(l, approx=True)
    return r * (2.0 - l * r)


def _kernel(x_hbm, k_hbm, v_hbm, wq_hbm, wo_hbm, wr_hbm, wg_hbm, wu_hbm, wd_hbm, c_hbm, wm_hbm,
            out_hbm,
            x_v, k_v, v_v, wq_v, wo_v, wr_v, wg_v, wu_v, wd_v, c_v, wm_v,
            h_v, h7_v, o7_v, o7a_v, q_v, qp_v, ost_v, bq_v, bo_v, acc_v, out_v, x1_v, h2_v, mod_v, best_v, besti_v, zero_v, zs_ref, sems):
    def cp(src, dst, i):
        return pltpu.make_async_copy(src, dst.bitcast(bf16), sems.at[i])

    def cp_rows(hbm, vm, r0, n, i):
        return cp(hbm.at[pl.ds(_mo(r0, n), n), :], vm.at[pl.ds(_mo(r0 // 2, n // 2), n // 2), :], i)

    def cp_cols(hbm, vm, c0, n, i):
        return cp(hbm.at[:, pl.ds(_mo(c0, 128), n)], vm.at[:, pl.ds(_mo(c0, 128), n)], i)

    def cp_wq(g, half):
        return cp_cols(wq_hbm, wq_v, g * GW + half * (GW // 2), GW // 2, S_WQ + 2 * g + half)

    def cp_k(g):
        return cp(k_hbm.at[g, pl.ds(SK - W, W), :], k_v.at[g], S_K + g)

    def cp_v(g):
        return cp(v_hbm.at[g, pl.ds(SK - W, W), :], v_v.at[g], S_V + g)

    def cp_x1(g, half):
        n = HM // HKV
        return cp_rows(x_hbm, x_v, TM + half * HM + g * n, n, S_X1 + 2 * g + half)


    def cp_wo(g):
        return cp_rows(wo_hbm, wo_v, g * GW, GW, S_WO + g)

    def cp_out(i):
        r0 = i * TM
        return pltpu.make_async_copy(out_v.at[pl.ds(_mo(r0 // 2, TM // 2), TM // 2), :].bitcast(bf16),
                                     out_hbm.at[pl.ds(_mo(r0, TM), TM), :], sems.at[S_OUT + i])

    cp_c = pltpu.make_async_copy(c_hbm, c_v, sems.at[S_C])
    cp_wr = pltpu.make_async_copy(wr_hbm, wr_v, sems.at[S_WR])
    cp_wms = cp_cols(wm_hbm, wm_v, 0, D, S_WMS)
    cp_wmc = cp_cols(wm_hbm, wm_v, D, D, S_WMC)
    cp_x0 = cp_rows(x_hbm, x_v, 0, TM, S_X0)
    cp_x2 = cp_rows(x_hbm, x_v, 2 * TM, S - 2 * TM, S_X2)

    def cp_wmb(n):
        return cp_cols(wm_hbm, wm_v, (2 + n) * D, D, S_WMB + n)

    def cp_ffn(n):
        return (cp_cols(wg_hbm, wg_v, n * FP, FP, S_WG + n), cp_cols(wu_hbm, wu_v, n * FP, FP, S_WU + n),
                cp_rows(wd_hbm, wd_v, n * FP, FP, S_WD + n))

    def group_set(g):
        return (cp_wq(g, 0), cp_x1(g, 0), cp_x1(g, 1), cp_wq(g, 1), cp_k(g), cp_v(g), cp_wo(g))


    cp_wq00 = cp_cols(wq_hbm, wq_v, 0, DH, S_WQ0)
    cp_wq01 = cp_cols(wq_hbm, wq_v, DH, GW // 2 - DH, S_WQ)
    for d in (cp_c, cp_wr, cp_x0, cp_wms, cp_wmc, cp_wq00, cp_wq01, cp_x1(0, 0), cp_x1(0, 1), cp_wq(0, 1),
              cp_k(0), cp_v(0), cp_wo(0)):
        d.start()
    best_v[...] = jnp.full(best_v.shape, -jnp.inf, f32)
    besti_v[...] = jnp.zeros(besti_v.shape, i32)
    zero_v[...] = jnp.zeros(zero_v.shape, u32)
    mod_v[...] = jnp.zeros(mod_v.shape, f32)
    q_v[0:8, 0:128] = jnp.zeros((8, 128), u32)
    qp_v[0:8, 0:128] = jnp.zeros((8, 128), f32)
    for n in range(8):
        zs_ref[n] = 0
    cp_c.wait()
    cp_wr.wait()
    cc = c_v[...].astype(f32)
    sc = jnp.broadcast_to((cc * jax.nn.sigmoid(cc)).astype(bf16), (16, D))
    cp_x0.wait()
    acc_v[1] = _ln(_bf(x_v[0:TM // 2, :]).astype(f32))
    cp_wms.wait()
    mod_v[:, 0:D] = jnp.dot(sc, _bf(wm_v[:, 0:D]), preferred_element_type=f32)[0:8]
    cp_wmc.wait()
    mod_v[:, D:2 * D] = jnp.dot(sc, _bf(wm_v[:, D:2 * D]), preferred_element_type=f32)[0:8]
    h_v[...] = _packs(acc_v[1] * (1.0 + mod_v[0:1, D:2 * D]) + mod_v[0:1, 0:D])

    def ln1_slice(row0, slot, dst0, normed=False, gate=None):
        sa = mod_v[0:1, 0 * D:1 * D]
        ca1 = 1.0 + mod_v[0:1, 1 * D:2 * D]
        if normed:
            xt, xb = acc_v[1, row0:row0 + 16, :], acc_v[1, row0 + HM:row0 + HM + 16, :]
            norm = lambda t: t
        else:
            xt, xb = (_bf(x_v[pl.ds(_mo(r // 2, 8), 8), :] | gate).astype(f32) for r in (row0, row0 + HM))
            norm = _ln
        dst = pl.ds(_mo(dst0 // 2, 8), 8)
        hs_ = []
        for r in (0, 8):
            top = norm(xt[r:r + 8]) * ca1 + sa
            bot = norm(xb[r:r + 8]) * ca1 + sa
            a11, a12, a21, a22 = top[:, :HK], top[:, HK:], bot[:, :HK], bot[:, HK:]
            hs_.append((a11 + a22, a21 + a22, a11, a22, a11 + a12, a21 - a11, a12 - a22))
        for n in range(7):
            h7_v[slot, n, dst, :] = pltpu.pack_elementwise([hs_[0][n], hs_[1][n]], packed_dtype=bf16)

    def wsum_slice(halves, dst):
        nr = dst.shape[1]
        for rr in range(0, nr, 8):
            for c in range(0, HK, 128):
                b11, b12, b21, b22 = (_halves(halves[kh][rr:rr + 8, nh * HK + c:nh * HK + c + 128])
                                      for kh in range(2) for nh in range(2))
                for n, (p, q, sign) in enumerate(((b11, b22, 1), (b12, b22, -1), (b21, b11, -1),
                                                  (b11, b12, 1), (b21, b22, 1))):
                    dst[n, rr:rr + 8, c:c + 128] = pltpu.pack_elementwise(
                        [u + w if sign > 0 else u - w for u, w in zip(p, q)], packed_dtype=bf16)

    def epi_rows16(src0, row0, slot, acc0, pos0, valid, gate):
        ga = mod_v[0:1, 2 * D:3 * D]
        sb = mod_v[0:1, 3 * D:4 * D]
        cb1 = 1.0 + mod_v[0:1, 4 * D:5 * D]
        gb = mod_v[0:1, 5 * D:6 * D]
        wr = wr_v[...].astype(f32).reshape(1, D)
        rows = pl.ds(_mo(row0 // 2, 8), 8)
        xw = x_v[pl.ds(_mo(src0 // 2, 8), 8), :]
        xs = _halves(xw if isinstance(gate, int) else xw | gate)
        x1s, outs, h2s = [], [], []
        for n in range(2):
            x1 = xs[n] + ga * acc_v[slot, pl.ds(_mo(acc0 + 8 * n, 8), 8), :]
            h2 = _ln(x1) * cb1 + sb
            x1s.append(x1)
            h2s.append(h2)
            outs.append(x1 + gb * h2)
            r = jnp.broadcast_to(jnp.sum(h2 * wr, axis=-1, keepdims=True), (8, 128))
            ib = row0 + n + 2 * lax.broadcasted_iota(i32, (8, 128), 0)
            sl = pl.ds(pos0 + 8 * n, 8)
            better = r > best_v[sl, :]
            if valid is not True:
                better = better & valid
            best_v[sl, :] = jnp.where(better, r, best_v[sl, :])
            besti_v[sl, :] = jnp.where(better, ib, besti_v[sl, :])
        x1_v[rows, :] = pltpu.pack_elementwise(x1s, packed_dtype=bf16)
        out_v[rows, :] = pltpu.pack_elementwise(outs, packed_dtype=bf16)
        h2_v[rows, :] = pltpu.pack_elementwise(h2s, packed_dtype=bf16)

    def wq_quad(g):
        def quad(kh, nh, r0=0, nr=HK // 2, c=0, nc=HK):
            return wq_v[pl.ds(_mo(kh * (HK // 2) + r0, 8), nr), pl.ds(_mo(g * GW + nh * HK + c, DH), nc)]
        return quad

    def wo_quad(g):
        def quad(kh, nh, r0=0, nr=HK // 2, c=0, nc=HK):
            return wo_v[pl.ds(_mo((g * GW + kh * HK) // 2 + r0, 8), nr), pl.ds(_mo(nh * HK + c, DH), nc)]
        return quad

    def b_operand(quad, sums, g, n, j):
        if n == 1:
            return quad(0, 0, c=j * DH, nc=DH)
        if n == 4:
            return quad(1, 1, c=j * DH, nc=DH)
        return sums[g, (0, None, 1, 2, None, 3, 4)[n], :, j * DH:(j + 1) * DH]

    def prep_part(g, part, do_q=True, do_o=True):
        nr = HK // 2 // WPARTS
        r0 = part * nr
        rows = pl.ds(_mo(r0, nr), nr)
        if do_q:
            wsum_slice([wq_v.at[pl.ds(_mo(kh * (HK // 2) + r0, nr), nr), pl.ds(_mo(g * GW, GW), GW)]
                        for kh in range(2)], bq_v.at[g, :, rows, :])
        if do_o:
            wsum_slice([wo_v.at[pl.ds(_mo((g * GW + kh * HK) // 2 + r0, nr), nr), :]
                        for kh in range(2)], bo_v.at[g, :, rows, :])

    def prep(g):
        lax.fori_loop(0, WPARTS, lambda part, _: prep_part(g, part), None)

    def period(i, g, mode):
        hs = i % 2
        if mode == 2:
            @pl.when(i == 0)
            def _():
                @pl.when(g < HKV - 1)
                def _():
                    for d in group_set(g + 1):
                        d.start()

                @pl.when(g == HKV - 1)
                def _():
                    cp_x2.start()
                cp_wmb(g).start()
                for d in group_set(g):
                    d.wait()
                prep(g)

            @pl.when((i == 1) & (g == 0))
            def _():
                for n in range(HKV):
                    cp_wmb(n).wait()
                cp_x2.wait()
                for part in range(WPARTS):
                    mc = slice(2 * D + part * (4 * D // WPARTS), 2 * D + (part + 1) * (4 * D // WPARTS))
                    mod_v[:, mc] = jnp.dot(sc, _bf(wm_v[:, mc]), preferred_element_type=f32)[0:8]
                    prep_part(0, part, do_o=False)

            @pl.when((g == 0) & (i >= 2))
            def _():
                cp_out(i - 2).start()

            piece = i * HKV + g - HKV

            @pl.when((piece >= 0) & (piece < NFP))
            def _():
                for d in cp_ffn(piece):
                    d.start()

        zero = zero_v[...]
        zz = [zs_ref[n] for n in range(8)]
        zs = zz[0]

        def ln_work(sub, dz):
            if mode == 0 and sub == 0:
                cp_x1(0, 0).wait()
                cp_x1(0, 1).wait()
            q0 = g * (HM // HKV) + sub * SR
            ln1_slice(jnp.minimum(i + 1, NB - 1) * TM + q0, 1 - hs, q0, gate=dz)
            return h7_v[1 - hs, 0, pl.ds(pl.multiple_of(q0 // 2 + zs, 8), 8), 0:128]

        def epi_work(sub, dz):
            toks = None
            for half in range(2):
                q0 = half * HM + g * (HM // HKV) + sub * SR
                src0 = jnp.maximum(i - 1, 0) * TM + q0
                row0 = jnp.where(i == 0, S, (i - 1) * TM) + q0
                pos = (2 * sub + half) * SR
                epi_rows16(src0, row0, 1 - hs, q0, pos, i > 0, dz)
                opq = pl.ds(pl.multiple_of(row0 // 2 + zs, 8), 8)
                ob = pl.ds(pl.multiple_of(pos + zs, 8), 8)
                t = (out_v[opq, 0:128] | x1_v[opq, 0:128]
                     | pltpu.bitcast(best_v[ob, :], u32) | pltpu.bitcast(besti_v[ob, :], u32))
                toks = t if toks is None else toks | t
            return toks

        early, late = [], []
        if mode == 2:
            for sub in range(NSL):
                early += [lambda dz, sub=sub: epi_work(sub, dz)] + [None] * (SIDE_STRIDE - 1)
                late += [lambda dz, sub=sub: ln_work(sub, dz)] + [None] * (SIDE_STRIDE - 1)
        else:
            def h7_first(n):
                ln1_slice(n * SR, 0, n * SR, normed=True)
                return h7_v[0, 0, pl.ds(pl.multiple_of(n * (SR // 2) + zs, 8), 8), 0:128]
            for sub in range(NSL):
                early.append(lambda dz, sub=sub: ln_work(sub, dz))
            for n in range(HM // SR):
                early.append(lambda dz, n=n: h7_first(n))
        pending = [None] * (SIDE_DIST if mode == 2 else 2)

        def anchored(w, extra=None):
            tok = pending.pop(0) if pending else None
            if extra is not None:
                tok = extra if tok is None else tok | extra
            if tok is not None:
                w = jnp.concatenate([w[0:8, :] | jnp.tile(tok & zero, (1, w.shape[1] // 128)), w[8:, :]], axis=0)
            return _bf(w)

        def after(res, queue):
            work = queue.pop(0) if queue else None
            if work is not None:
                src = (qp_v.at[:, 0:128] if queue is early else acc_v.at[hs, :, 0:128]) if mode == 2 else q_v.at[:, 0:128]
                gate = pltpu.bitcast(src[pl.ds(pl.multiple_of(zs, 8), 8), :], u32) & zero
                pending.append(work(jnp.tile(gate, (1, D // 128))))
            else:
                pending.append(None)

        def mm(a, w, queue, extra=None):
            res = jnp.dot(a, anchored(w, extra), preferred_element_type=f32)
            after(res, queue)
            return res

        if mode == 0:
            for hh in range(REP):
                if hh == 0:
                    cp_wq00.wait()
                elif hh == 1:
                    cp_wq01.wait()
                elif hh == REP // 2:
                    cp_wq(0, 1).wait()
                h = _bf(h_v[pl.ds(pl.multiple_of(zz[hh], 8), TM // 2), :])
                qh = mm(h, wq_v[:, pl.ds(_mo(g * GW + hh * DH, DH), DH)], early)
                q_v[:, hh * DH:(hh + 1) * DH] = _packs(qh * QSCALE)
        else:
            quad = wq_quad(g)
            for j in range(HK // DH):
                def d(n):
                    return mm(_bf(h7_v[hs + zz[j], n]), b_operand(quad, bq_v, g, n, j), early)
                L, R = pl.ds(0, DH), pl.ds(DH, DH)
                QL, QR_ = pl.ds(j * DH, DH), pl.ds(HK + j * DH, DH)
                def comb(m, *ops):
                    for r in range(0, HM, CR):
                        mc = m[r:r + CR]
                        for (row, col, kind, qsrc) in ops:
                            rows = pl.ds(row + r, CR)
                            if kind == "set":
                                qp_v[rows, col] = mc
                            elif kind == "add":
                                qp_v[rows, col] += mc
                            elif kind == "sub":
                                qp_v[rows, col] -= mc
                            else:
                                q_v[pl.ds((row + r) // 2, CR // 2), qsrc] = _packs((qp_v[rows, col] + mc) * QSCALE)
                comb(d(0), (0, L, "set", None), (HM, R, "set", None))
                comb(d(1), (HM, R, "sub", None), (HM, L, "set", None))
                comb(d(2), (HM, R, "add", None), (0, R, "set", None))
                comb(d(3), (0, L, "add", None), (HM, L, "q", QL))
                comb(d(4), (0, L, "sub", None), (0, R, "q", QR_))
                comb(d(5), (HM, R, "q", QR_))
                comb(d(6), (0, L, "q", QL))

        if mode == 0:
            cp_k(0).wait()
            cp_v(0).wait()
            for d in group_set(1) + (cp_wmb(0),):
                d.start()
        otok = None
        for hh in range(REP):
            s = lax.dot_general(_bf(q_v[:, hh * DH:(hh + 1) * DH]), anchored(k_v[g]), (((1,), (1,)), ((), ())), preferred_element_type=f32)
            after(s, early)
            m = jnp.max(s, axis=-1, keepdims=True)
            p = jnp.exp2(s - m)
            l = jnp.sum(p, axis=-1, keepdims=True)
            o = mm(p.astype(bf16), v_v[g], early, otok) * _recip(l)
            col = slice((hh % 4) * DH, (hh % 4 + 1) * DH)
            if hh < 4:
                top, bot = o[:HM], o[HM:]
                ost_v[:, col] = o
                o7a_v[0, :, col] = _packs(top)
                o7a_v[1, :, col] = _packs(bot - top)
                oref = o7a_v.at[1]
            else:
                a12, a22 = o[:HM], o[HM:]
                a11, a21 = ost_v[0:HM, col], ost_v[HM:TM, col]
                o7_v[0, :, col] = _packs(a11 + a22)
                o7_v[1, :, col] = _packs(a21 + a22)
                o7_v[2, :, col] = _packs(a22)
                o7_v[3, :, col] = _packs(a11 + a12)
                o7_v[4, :, col] = _packs(a12 - a22)
                oref = o7_v.at[4]
            otok = None
            if hh + 2 < REP:
                cc = (hh % 4) * DH
                otok = oref[pl.ds(pl.multiple_of(zs, 8), 8), pl.ds(pl.multiple_of(cc + zs * 128, DH), DH)]

        if mode == 0:
            cp_wo(0).wait()
            lax.fori_loop(0, WPARTS, lambda part, _: prep_part(0, part, do_q=False), None)
        quad = wo_quad(g)

        def d(n, j):
            if n in (2, 5):
                lhs = o7a_v[(0 if n == 2 else 1) + zz[j]]
            else:
                lhs = o7_v[(0, 1, None, 2, 3, None, 4)[n] + zz[j]]
            return mm(_bf(lhs), b_operand(quad, bo_v, g, n, j), late)

        def comb(m, j, *ops):
            for r in range(0, HM, CR):
                mc = m[r:r + CR]
                for (row, right, kind) in ops:
                    rows, col = pl.ds(row + r, CR), pl.ds(right * HK + j * DH, DH)
                    if kind == "first" and mode == 0:
                        acc_v[hs, rows, col] = mc
                    elif kind == "first":
                        acc_v[hs, rows, col] = jnp.where(g == 0, mc, acc_v[hs, rows, col] + mc)
                    elif kind == "add":
                        acc_v[hs, rows, col] += mc
                    else:
                        acc_v[hs, rows, col] -= mc
        for j in range(HK // DH):
            comb(d(2, j), j, (HM, 1, "first"), (0, 1, "first"))
            comb(d(5, j), j, (HM, 1, "add"))
        for j in range(HK // DH):
            comb(d(0, j), j, (0, 0, "first"), (HM, 1, "add"))
            comb(d(1, j), j, (HM, 1, "sub"), (HM, 0, "first"))
            comb(d(3, j), j, (0, 0, "add"), (HM, 0, "add"))
            comb(d(4, j), j, (0, 0, "sub"), (0, 1, "add"))
            comb(d(6, j), j, (0, 0, "add"))
        assert not any(early) and not any(late)

    with jax.named_scope("p00"):
        period(0, 0, 0)
    with jax.named_scope("loopB"):
        def step_b(t, _):
            period(t // HKV, t % HKV, 2)
        lax.fori_loop(1, NB * HKV, step_b, None)
    cp_out(NB - 2).start()

    with jax.named_scope("tail"):
        ga, sb, cb, gb = (mod_v[0:1, n * D:(n + 1) * D] for n in range(2, 6))
        wr = wr_v[...].astype(f32).reshape(1, D)
        last = pl.ds((NB - 1) * TM // 2, TM // 2)
        x1 = _unpacks(x_v[last, :]) + ga * acc_v[(NB - 1) % 2]
        x1_v[last, :] = _packs(x1)
        h2 = _ln(x1) * (1.0 + cb) + sb
        out_v[last, :] = _packs(x1 + gb * h2)
        h2_v[last, :] = _packs(h2)
        cp_out(NB - 1).start()
        r = jnp.broadcast_to(jnp.sum(h2 * wr, axis=-1, keepdims=True), (TM, 128))
        pos = lax.broadcasted_iota(i32, (QR, 128), 0)
        pos = (pos & ~15) + 2 * (pos & 7) + ((pos & 15) >> 3)
        for qd in range(HKV):
            rb = r[qd * QR:(qd + 1) * QR]
            better = rb > best_v[...]
            best_v[...] = jnp.where(better, rb, best_v[...])
            besti_v[...] = jnp.where(better, (NB - 1) * TM + qd * QR + pos, besti_v[...])
        bv = best_v[...]
        mx = jnp.max(bv, axis=0, keepdims=True)
        idx = jnp.min(jnp.where(bv == mx, besti_v[...], S), axis=0, keepdims=True)[0, 0]
        idx = jnp.minimum(idx, S - 1)
        base = pl.multiple_of((idx // 16) * 16, 16)
        pb = pl.ds(pl.multiple_of(base // 2, 8), 8)
        x1 = _bf(x1_v[pb, :]).astype(f32)
        hsel = _bf(h2_v[pb, :])
        h2 = hsel.astype(f32)
        r_sel = mx[:, 0:1]
        for n in range(NFP):
            for d in cp_ffn(n):
                d.wait()
        acts, y = [], None
        for n in range(NFP + 1):
            if n < NFP:
                cols = slice(n * FP, (n + 1) * FP)
                gg = jnp.dot(hsel, _bf(wg_v[:, cols]), preferred_element_type=f32)
                uu = jnp.dot(hsel, _bf(wu_v[:, cols]), preferred_element_type=f32)
                acts.append((gg * jax.nn.sigmoid(gg) * uu).astype(bf16))
            if n > 0:
                part = jnp.dot(acts[n - 1], _bf(wd_v[(n - 1) * FP // 2:n * FP // 2, :]), preferred_element_type=f32)
                y = part if y is None else y + part
        y = y * jax.nn.sigmoid(r_sel)
        rows = base + lax.broadcasted_iota(i32, (16, D), 0)
        new = (x1 + gb * (h2 + y)).astype(bf16)
        for i in range(NB):
            cp_out(i).wait()
        out_v[pb, :] = pltpu.bitcast(jnp.where(rows == idx, new, _bf(out_v[pb, :])), u32)
        fin = pltpu.make_async_copy(out_v.at[pb, :].bitcast(bf16), out_hbm.at[pl.ds(base, 16), :], sems.at[S_FIN])
        fin.start()
        fin.wait()


@jax.jit
def pallas_adaLN_cond__sliding_block_cached__moe_arch_mod__prompt_kernel(
    A_x, A_k_cache, A_v_cache, A_wq, A_wo, B_x, B_w_r, B_w_gate, B_w_up, B_w_down, c, w_mod,
):
    anyspec = pl.BlockSpec(memory_space=pl.ANY)
    out = pl.pallas_call(
        _kernel,
        out_shape=jax.ShapeDtypeStruct((S, D), bf16),
        in_specs=[anyspec] * 11,
        out_specs=anyspec,
        scratch_shapes=[
            pltpu.VMEM((S // 2, D), u32),
            pltpu.VMEM((HKV, W // 2, DH), u32),
            pltpu.VMEM((HKV, W // 2, DH), u32),
            pltpu.VMEM((D // 2, HQ * DH), u32),
            pltpu.VMEM((HQ * DH // 2, D), u32),
            pltpu.VMEM((D,), bf16),
            pltpu.VMEM((D // 2, F), u32),
            pltpu.VMEM((D // 2, F), u32),
            pltpu.VMEM((F // 2, D), u32),
            pltpu.VMEM((1, D), bf16),
            pltpu.VMEM((D // 2, 6 * D), u32),
            pltpu.VMEM((TM // 2, D), u32),
            pltpu.VMEM((2, 7, HM // 2, HK), u32),
            pltpu.VMEM((5, HM // 2, HK), u32),
            pltpu.VMEM((2, HM // 2, HK), u32),
            pltpu.VMEM((TM // 2, GW), u32),
            pltpu.VMEM((TM, 2 * DH), f32),
            pltpu.VMEM((TM, HK), f32),
            pltpu.VMEM((HKV, 5, HK // 2, HK), u32),
            pltpu.VMEM((HKV, 5, HK // 2, HK), u32),
            pltpu.VMEM((2, TM, D), f32),
            pltpu.VMEM((S // 2 + TM // 2, D), u32),
            pltpu.VMEM((S // 2 + TM // 2, D), u32),
            pltpu.VMEM((S // 2 + TM // 2, D), u32),
            pltpu.VMEM((8, 6 * D), f32),
            pltpu.VMEM((QR, 128), f32),
            pltpu.VMEM((QR, 128), i32),
            pltpu.VMEM((8, 128), u32),
            pltpu.SMEM((8,), i32),
            pltpu.SemaphoreType.DMA((NSEM,)),
        ],
        compiler_params=pltpu.CompilerParams(vmem_limit_bytes=120 * 1024 * 1024),
    )(
        A_x.reshape(S, D), A_k_cache.reshape(HKV, SK, DH), A_v_cache.reshape(HKV, SK, DH),
        A_wq, A_wo, B_w_r, B_w_gate, B_w_up, B_w_down, c, w_mod,
    )
    return out.reshape(1, S, D)
```

```python
import jax
import jax.numpy as jnp
from jax import lax
import jax.experimental.pallas as pl
import jax.experimental.pallas.tpu as pltpu

S, D, HQ, HKV, DH, SK, W, F = 2048, 1024, 32, 4, 128, 2048, 512, 3584
REP = HQ // HKV
GW = REP * DH
TM = 512
NB = S // TM
QR = TM // HKV
HM = TM // 2
HK = D // 2
WPARTS = 8
SIDE_STRIDE = 7
SIDE_DIST = 4
CR = 32
SR = 16
NSL = HM // HKV // SR
LOG2E = 1.4426950408889634
QSCALE = (DH ** -0.5) * LOG2E
EPS = 1e-5
f32, bf16, u32, i32 = jnp.float32, jnp.bfloat16, jnp.uint32, jnp.int32

S_C, S_WMS, S_WMC, S_X0, S_X2, S_WR, S_FIN, S_WQ0 = range(8)
S_WQ = 8
S_WO = S_WQ + 2 * HKV
S_K = S_WO + HKV
S_V = S_K + HKV
S_X1 = S_V + HKV
S_WMB = S_X1 + 2 * HKV
S_OUT = S_WMB + HKV
NFP = 7
FP = F // NFP
S_WG = S_OUT + NB
S_WU = S_WG + NFP
S_WD = S_WU + NFP
NSEM = S_WD + NFP


def _ln(x):
    m = jnp.mean(x, axis=-1, keepdims=True)
    xc = x - m
    v = jnp.mean(xc * xc, axis=-1, keepdims=True)
    return xc * lax.rsqrt(v + EPS)


def _packs(y):
    r, c = y.shape
    y4 = y.reshape(r // 16, 2, 8, c)
    return pltpu.pack_elementwise([y4[:, 0].reshape(r // 2, c), y4[:, 1].reshape(r // 2, c)], packed_dtype=bf16)


def _halves(w):
    return tuple(pltpu.unpack_elementwise(w, index=n, packed_dtype=bf16, unpacked_dtype=f32) for n in range(2))


def _unpacks(w):
    r, c = w.shape
    lo, hi = (t.reshape(r // 8, 8, c) for t in _halves(w))
    return jnp.stack([lo, hi], axis=1).reshape(2 * r, c)


def _bf(x):
    return pltpu.bitcast(x, bf16)


def _mo(x, m):
    return x if isinstance(x, int) else pl.multiple_of(x, m)


def _recip(l):
    r = pl.reciprocal(l, approx=True)
    return r * (2.0 - l * r)


def _kernel(x_hbm, k_hbm, v_hbm, wq_hbm, wo_hbm, wr_hbm, wg_hbm, wu_hbm, wd_hbm, c_hbm, wm_hbm,
            out_hbm,
            x_v, k_v, v_v, wq_v, wo_v, wr_v, wg_v, wu_v, wd_v, c_v, wm_v,
            h_v, h7_v, o7_v, o7a_v, q_v, qp_v, ost_v, bq_v, bo_v, acc_v, out_v, x1_v, h2_v, mod_v, best_v, besti_v, zero_v, zs_ref, sems):
    def cp(src, dst, i):
        return pltpu.make_async_copy(src, dst.bitcast(bf16), sems.at[i])

    def cp_rows(hbm, vm, r0, n, i):
        return cp(hbm.at[pl.ds(_mo(r0, n), n), :], vm.at[pl.ds(_mo(r0 // 2, n // 2), n // 2), :], i)

    def cp_cols(hbm, vm, c0, n, i):
        return cp(hbm.at[:, pl.ds(_mo(c0, 128), n)], vm.at[:, pl.ds(_mo(c0, 128), n)], i)

    def cp_wq(g, half):
        return cp_cols(wq_hbm, wq_v, g * GW + half * (GW // 2), GW // 2, S_WQ + 2 * g + half)

    def cp_k(g):
        return cp(k_hbm.at[g, pl.ds(SK - W, W), :], k_v.at[g], S_K + g)

    def cp_v(g):
        return cp(v_hbm.at[g, pl.ds(SK - W, W), :], v_v.at[g], S_V + g)

    def cp_x1(g, half):
        n = HM // HKV
        return cp_rows(x_hbm, x_v, TM + half * HM + g * n, n, S_X1 + 2 * g + half)


    def cp_wo(g):
        return cp_rows(wo_hbm, wo_v, g * GW, GW, S_WO + g)

    def cp_out(i):
        r0 = i * TM
        return pltpu.make_async_copy(out_v.at[pl.ds(_mo(r0 // 2, TM // 2), TM // 2), :].bitcast(bf16),
                                     out_hbm.at[pl.ds(_mo(r0, TM), TM), :], sems.at[S_OUT + i])

    cp_c = pltpu.make_async_copy(c_hbm, c_v, sems.at[S_C])
    cp_wr = pltpu.make_async_copy(wr_hbm, wr_v, sems.at[S_WR])
    cp_wms = cp_cols(wm_hbm, wm_v, 0, D, S_WMS)
    cp_wmc = cp_cols(wm_hbm, wm_v, D, D, S_WMC)
    cp_x0 = cp_rows(x_hbm, x_v, 0, TM, S_X0)
    cp_x2 = cp_rows(x_hbm, x_v, 2 * TM, S - 2 * TM, S_X2)

    def cp_wmb(n):
        return cp_cols(wm_hbm, wm_v, (2 + n) * D, D, S_WMB + n)

    def cp_ffn(n):
        return (cp_cols(wg_hbm, wg_v, n * FP, FP, S_WG + n), cp_cols(wu_hbm, wu_v, n * FP, FP, S_WU + n),
                cp_rows(wd_hbm, wd_v, n * FP, FP, S_WD + n))

    def group_set(g):
        return (cp_wq(g, 0), cp_x1(g, 0), cp_x1(g, 1), cp_wq(g, 1), cp_k(g), cp_v(g), cp_wo(g))


    cp_wq00 = cp_cols(wq_hbm, wq_v, 0, DH, S_WQ0)
    cp_wq01 = cp_cols(wq_hbm, wq_v, DH, GW // 2 - DH, S_WQ)
    for d in (cp_c, cp_wr, cp_x0, cp_wms, cp_wmc, cp_wq00, cp_wq01, cp_x1(0, 0), cp_x1(0, 1), cp_wq(0, 1),
              cp_k(0), cp_v(0), cp_wo(0)):
        d.start()
    best_v[...] = jnp.full(best_v.shape, -jnp.inf, f32)
    besti_v[...] = jnp.zeros(besti_v.shape, i32)
    zero_v[...] = jnp.zeros(zero_v.shape, u32)
    mod_v[...] = jnp.zeros(mod_v.shape, f32)
    q_v[0:8, 0:128] = jnp.zeros((8, 128), u32)
    qp_v[0:8, 0:128] = jnp.zeros((8, 128), f32)
    for n in range(8):
        zs_ref[n] = 0
    cp_c.wait()
    cp_wr.wait()
    cc = c_v[...].astype(f32)
    sc = jnp.broadcast_to((cc * jax.nn.sigmoid(cc)).astype(bf16), (16, D))
    cp_x0.wait()
    acc_v[1] = _ln(_bf(x_v[0:TM // 2, :]).astype(f32))
    cp_wms.wait()
    mod_v[:, 0:D] = jnp.dot(sc, _bf(wm_v[:, 0:D]), preferred_element_type=f32)[0:8]
    cp_wmc.wait()
    mod_v[:, D:2 * D] = jnp.dot(sc, _bf(wm_v[:, D:2 * D]), preferred_element_type=f32)[0:8]
    h_v[...] = _packs(acc_v[1] * (1.0 + mod_v[0:1, D:2 * D]) + mod_v[0:1, 0:D])

    def ln1_slice(row0, slot, dst0, normed=False, gate=None):
        sa = mod_v[0:1, 0 * D:1 * D]
        ca1 = 1.0 + mod_v[0:1, 1 * D:2 * D]
        if normed:
            xt, xb = acc_v[1, row0:row0 + 16, :], acc_v[1, row0 + HM:row0 + HM + 16, :]
            norm = lambda t: t
        else:
            xt, xb = (_bf(x_v[pl.ds(_mo(r // 2, 8), 8), :] | gate).astype(f32) for r in (row0, row0 + HM))
            norm = _ln
        dst = pl.ds(_mo(dst0 // 2, 8), 8)
        hs_ = []
        for r in (0, 8):
            top = norm(xt[r:r + 8]) * ca1 + sa
            bot = norm(xb[r:r + 8]) * ca1 + sa
            a11, a12, a21, a22 = top[:, :HK], top[:, HK:], bot[:, :HK], bot[:, HK:]
            hs_.append((a11 + a22, a21 + a22, a11, a22, a11 + a12, a21 - a11, a12 - a22))
        for n in range(7):
            h7_v[slot, n, dst, :] = pltpu.pack_elementwise([hs_[0][n], hs_[1][n]], packed_dtype=bf16)

    def wsum_slice(halves, dst):
        nr = dst.shape[1]
        for rr in range(0, nr, 8):
            for c in range(0, HK, 128):
                b11, b12, b21, b22 = (_halves(halves[kh][rr:rr + 8, nh * HK + c:nh * HK + c + 128])
                                      for kh in range(2) for nh in range(2))
                for n, (p, q, sign) in enumerate(((b11, b22, 1), (b12, b22, -1), (b21, b11, -1),
                                                  (b11, b12, 1), (b21, b22, 1))):
                    dst[n, rr:rr + 8, c:c + 128] = pltpu.pack_elementwise(
                        [u + w if sign > 0 else u - w for u, w in zip(p, q)], packed_dtype=bf16)

    def epi_rows16(src0, row0, slot, acc0, pos0, valid, gate):
        ga = mod_v[0:1, 2 * D:3 * D]
        sb = mod_v[0:1, 3 * D:4 * D]
        cb1 = 1.0 + mod_v[0:1, 4 * D:5 * D]
        gb = mod_v[0:1, 5 * D:6 * D]
        wr = wr_v[...].astype(f32).reshape(1, D)
        rows = pl.ds(_mo(row0 // 2, 8), 8)
        xw = x_v[pl.ds(_mo(src0 // 2, 8), 8), :]
        xs = _halves(xw if isinstance(gate, int) else xw | gate)
        x1s, outs, h2s = [], [], []
        for n in range(2):
            x1 = xs[n] + ga * acc_v[slot, pl.ds(_mo(acc0 + 8 * n, 8), 8), :]
            h2 = _ln(x1) * cb1 + sb
            x1s.append(x1)
            h2s.append(h2)
            outs.append(x1 + gb * h2)
            r = jnp.broadcast_to(jnp.sum(h2 * wr, axis=-1, keepdims=True), (8, 128))
            ib = row0 + n + 2 * lax.broadcasted_iota(i32, (8, 128), 0)
            sl = pl.ds(pos0 + 8 * n, 8)
            better = r > best_v[sl, :]
            if valid is not True:
                better = better & valid
            best_v[sl, :] = jnp.where(better, r, best_v[sl, :])
            besti_v[sl, :] = jnp.where(better, ib, besti_v[sl, :])
        x1_v[rows, :] = pltpu.pack_elementwise(x1s, packed_dtype=bf16)
        out_v[rows, :] = pltpu.pack_elementwise(outs, packed_dtype=bf16)
        h2_v[rows, :] = pltpu.pack_elementwise(h2s, packed_dtype=bf16)

    def wq_quad(g):
        def quad(kh, nh, r0=0, nr=HK // 2, c=0, nc=HK):
            return wq_v[pl.ds(_mo(kh * (HK // 2) + r0, 8), nr), pl.ds(_mo(g * GW + nh * HK + c, DH), nc)]
        return quad

    def wo_quad(g):
        def quad(kh, nh, r0=0, nr=HK // 2, c=0, nc=HK):
            return wo_v[pl.ds(_mo((g * GW + kh * HK) // 2 + r0, 8), nr), pl.ds(_mo(nh * HK + c, DH), nc)]
        return quad

    def b_operand(quad, sums, g, n, j):
        if n == 1:
            return quad(0, 0, c=j * DH, nc=DH)
        if n == 4:
            return quad(1, 1, c=j * DH, nc=DH)
        return sums[g, (0, None, 1, 2, None, 3, 4)[n], :, j * DH:(j + 1) * DH]

    def prep_part(g, part, do_q=True, do_o=True):
        nr = HK // 2 // WPARTS
        r0 = part * nr
        rows = pl.ds(_mo(r0, nr), nr)
        if do_q:
            wsum_slice([wq_v.at[pl.ds(_mo(kh * (HK // 2) + r0, nr), nr), pl.ds(_mo(g * GW, GW), GW)]
                        for kh in range(2)], bq_v.at[g, :, rows, :])
        if do_o:
            wsum_slice([wo_v.at[pl.ds(_mo((g * GW + kh * HK) // 2 + r0, nr), nr), :]
                        for kh in range(2)], bo_v.at[g, :, rows, :])

    def period(i, g, mode):
        hs = i % 2
        if mode == 2:
            @pl.when(i == 0)
            def _():
                @pl.when(g < HKV - 1)
                def _():
                    for d in group_set(g + 1):
                        d.start()

                @pl.when(g == HKV - 1)
                def _():
                    cp_x2.start()
                cp_wmb(g).start()
                for d in group_set(g):
                    d.wait()
                cp_wmb(g - 1).wait()
                for part in range(WPARTS):
                    mc = pl.ds(pl.multiple_of((1 + g) * D + part * (D // WPARTS), DH), D // WPARTS)
                    mod_v[:, mc] = jnp.dot(sc, _bf(wm_v[:, mc]), preferred_element_type=f32)[0:8]
                    prep_part(g, part)

            @pl.when((i == 1) & (g == 0))
            def _():
                cp_wmb(HKV - 1).wait()
                cp_x2.wait()
                for part in range(WPARTS):
                    mc = slice(5 * D + part * (D // WPARTS), 5 * D + (part + 1) * (D // WPARTS))
                    mod_v[:, mc] = jnp.dot(sc, _bf(wm_v[:, mc]), preferred_element_type=f32)[0:8]
                    prep_part(0, part, do_o=False)

            @pl.when((g == 0) & (i >= 2))
            def _():
                cp_out(i - 2).start()

            piece = i * HKV + g - HKV

            @pl.when((piece >= 0) & (piece < NFP))
            def _():
                for d in cp_ffn(piece):
                    d.start()

        zero = zero_v[...]
        zz = [zs_ref[n] for n in range(8)]
        zs = zz[0]

        def ln_work(sub, dz):
            if mode == 0 and sub == 0:
                cp_x1(0, 0).wait()
                cp_x1(0, 1).wait()
            q0 = g * (HM // HKV) + sub * SR
            ln1_slice(jnp.minimum(i + 1, NB - 1) * TM + q0, 1 - hs, q0, gate=dz)
            return h7_v[1 - hs, 0, pl.ds(pl.multiple_of(q0 // 2 + zs, 8), 8), 0:128]

        def epi_work(sub, dz):
            toks = None
            for half in range(2):
                q0 = half * HM + g * (HM // HKV) + sub * SR
                src0 = jnp.maximum(i - 1, 0) * TM + q0
                row0 = jnp.where(i == 0, S, (i - 1) * TM) + q0
                pos = (2 * sub + half) * SR
                epi_rows16(src0, row0, 1 - hs, q0, pos, i > 0, dz)
                opq = pl.ds(pl.multiple_of(row0 // 2 + zs, 8), 8)
                ob = pl.ds(pl.multiple_of(pos + zs, 8), 8)
                t = (out_v[opq, 0:128] | x1_v[opq, 0:128]
                     | pltpu.bitcast(best_v[ob, :], u32) | pltpu.bitcast(besti_v[ob, :], u32))
                toks = t if toks is None else toks | t
            return toks

        early, late = [], []
        if mode == 2:
            for sub in range(NSL):
                early += [lambda dz, sub=sub: epi_work(sub, dz)] + [None] * (SIDE_STRIDE - 1)
                late += [lambda dz, sub=sub: ln_work(sub, dz)] + [None] * (SIDE_STRIDE - 1)
        else:
            def h7_first(n):
                ln1_slice(n * SR, 0, n * SR, normed=True)
                return h7_v[0, 0, pl.ds(pl.multiple_of(n * (SR // 2) + zs, 8), 8), 0:128]
            for sub in range(NSL):
                early.append(lambda dz, sub=sub: ln_work(sub, dz))
            for n in range(HM // SR):
                early.append(lambda dz, n=n: h7_first(n))
        pending = [None] * (SIDE_DIST if mode == 2 else 2)

        def anchored(w, extra=None):
            tok = pending.pop(0) if pending else None
            if extra is not None:
                tok = extra if tok is None else tok | extra
            if tok is not None:
                w = jnp.concatenate([w[0:8, :] | jnp.tile(tok & zero, (1, w.shape[1] // 128)), w[8:, :]], axis=0)
            return _bf(w)

        def after(res, queue):
            work = queue.pop(0) if queue else None
            if work is not None:
                src = (qp_v.at[:, 0:128] if queue is early else acc_v.at[hs, :, 0:128]) if mode == 2 else q_v.at[:, 0:128]
                gate = pltpu.bitcast(src[pl.ds(pl.multiple_of(zs, 8), 8), :], u32) & zero
                pending.append(work(jnp.tile(gate, (1, D // 128))))
            else:
                pending.append(None)

        def mm(a, w, queue, extra=None):
            res = jnp.dot(a, anchored(w, extra), preferred_element_type=f32)
            after(res, queue)
            return res

        if mode == 0:
            for hh in range(REP):
                if hh == 0:
                    cp_wq00.wait()
                elif hh == 1:
                    cp_wq01.wait()
                elif hh == REP // 2:
                    cp_wq(0, 1).wait()
                h = _bf(h_v[pl.ds(pl.multiple_of(zz[hh], 8), TM // 2), :])
                qh = mm(h, wq_v[:, pl.ds(_mo(g * GW + hh * DH, DH), DH)], early)
                q_v[:, hh * DH:(hh + 1) * DH] = _packs(qh * QSCALE)
        else:
            quad = wq_quad(g)
            for j in range(HK // DH):
                def d(n):
                    return mm(_bf(h7_v[hs + zz[j], n]), b_operand(quad, bq_v, g, n, j), early)
                L, R = pl.ds(0, DH), pl.ds(DH, DH)
                QL, QR_ = pl.ds(j * DH, DH), pl.ds(HK + j * DH, DH)
                def comb(m, *ops):
                    for r in range(0, HM, CR):
                        mc = m[r:r + CR]
                        for (row, col, kind, qsrc) in ops:
                            rows = pl.ds(row + r, CR)
                            if kind == "set":
                                qp_v[rows, col] = mc
                            elif kind == "add":
                                qp_v[rows, col] += mc
                            elif kind == "sub":
                                qp_v[rows, col] -= mc
                            else:
                                q_v[pl.ds((row + r) // 2, CR // 2), qsrc] = _packs((qp_v[rows, col] + mc) * QSCALE)
                comb(d(0), (0, L, "set", None), (HM, R, "set", None))
                comb(d(1), (HM, R, "sub", None), (HM, L, "set", None))
                comb(d(2), (HM, R, "add", None), (0, R, "set", None))
                comb(d(3), (0, L, "add", None), (HM, L, "q", QL))
                comb(d(4), (0, L, "sub", None), (0, R, "q", QR_))
                comb(d(5), (HM, R, "q", QR_))
                comb(d(6), (0, L, "q", QL))

        if mode == 0:
            cp_k(0).wait()
            cp_v(0).wait()
            for d in group_set(1) + (cp_wmb(0),):
                d.start()
        otok = None
        for hh in range(REP):
            s = lax.dot_general(_bf(q_v[:, hh * DH:(hh + 1) * DH]), anchored(k_v[g]), (((1,), (1,)), ((), ())), preferred_element_type=f32)
            after(s, early)
            m = jnp.max(s, axis=-1, keepdims=True)
            p = jnp.exp2(s - m)
            l = jnp.sum(p, axis=-1, keepdims=True)
            o = mm(p.astype(bf16), v_v[g], early, otok) * _recip(l)
            col = slice((hh % 4) * DH, (hh % 4 + 1) * DH)
            if hh < 4:
                top, bot = o[:HM], o[HM:]
                ost_v[:, col] = o
                o7a_v[0, :, col] = _packs(top)
                o7a_v[1, :, col] = _packs(bot - top)
                oref = o7a_v.at[1]
            else:
                a12, a22 = o[:HM], o[HM:]
                a11, a21 = ost_v[0:HM, col], ost_v[HM:TM, col]
                o7_v[0, :, col] = _packs(a11 + a22)
                o7_v[1, :, col] = _packs(a21 + a22)
                o7_v[2, :, col] = _packs(a22)
                o7_v[3, :, col] = _packs(a11 + a12)
                o7_v[4, :, col] = _packs(a12 - a22)
                oref = o7_v.at[4]
            otok = None
            if hh + 2 < REP:
                cc = (hh % 4) * DH
                otok = oref[pl.ds(pl.multiple_of(zs, 8), 8), pl.ds(pl.multiple_of(cc + zs * 128, DH), DH)]

        if mode == 0:
            cp_wo(0).wait()
            lax.fori_loop(0, WPARTS, lambda part, _: prep_part(0, part, do_q=False), None)
        quad = wo_quad(g)

        def d(n, j):
            if n in (2, 5):
                lhs = o7a_v[(0 if n == 2 else 1) + zz[j]]
            else:
                lhs = o7_v[(0, 1, None, 2, 3, None, 4)[n] + zz[j]]
            return mm(_bf(lhs), b_operand(quad, bo_v, g, n, j), late)

        def comb(m, j, *ops):
            for r in range(0, HM, CR):
                mc = m[r:r + CR]
                for (row, right, kind) in ops:
                    rows, col = pl.ds(row + r, CR), pl.ds(right * HK + j * DH, DH)
                    if kind == "first" and mode == 0:
                        acc_v[hs, rows, col] = mc
                    elif kind == "first":
                        acc_v[hs, rows, col] = jnp.where(g == 0, mc, acc_v[hs, rows, col] + mc)
                    elif kind == "add":
                        acc_v[hs, rows, col] += mc
                    else:
                        acc_v[hs, rows, col] -= mc
        for j in range(HK // DH):
            comb(d(2, j), j, (HM, 1, "first"), (0, 1, "first"))
            comb(d(5, j), j, (HM, 1, "add"))
        for j in range(HK // DH):
            comb(d(0, j), j, (0, 0, "first"), (HM, 1, "add"))
            comb(d(1, j), j, (HM, 1, "sub"), (HM, 0, "first"))
            comb(d(3, j), j, (0, 0, "add"), (HM, 0, "add"))
            comb(d(4, j), j, (0, 0, "sub"), (0, 1, "add"))
            comb(d(6, j), j, (0, 0, "add"))
        assert not any(early) and not any(late)

    with jax.named_scope("p00"):
        period(0, 0, 0)
    with jax.named_scope("loopB"):
        def step_b(t, _):
            period(t // HKV, t % HKV, 2)
        lax.fori_loop(1, NB * HKV, step_b, None)
    cp_out(NB - 2).start()

    with jax.named_scope("tail"):
        ga, sb, cb, gb = (mod_v[0:1, n * D:(n + 1) * D] for n in range(2, 6))
        wr = wr_v[...].astype(f32).reshape(1, D)
        last = pl.ds((NB - 1) * TM // 2, TM // 2)
        x1 = _unpacks(x_v[last, :]) + ga * acc_v[(NB - 1) % 2]
        x1_v[last, :] = _packs(x1)
        h2 = _ln(x1) * (1.0 + cb) + sb
        out_v[last, :] = _packs(x1 + gb * h2)
        h2_v[last, :] = _packs(h2)
        cp_out(NB - 1).start()
        r = jnp.broadcast_to(jnp.sum(h2 * wr, axis=-1, keepdims=True), (TM, 128))
        pos = lax.broadcasted_iota(i32, (QR, 128), 0)
        pos = (pos & ~15) + 2 * (pos & 7) + ((pos & 15) >> 3)
        for qd in range(HKV):
            rb = r[qd * QR:(qd + 1) * QR]
            better = rb > best_v[...]
            best_v[...] = jnp.where(better, rb, best_v[...])
            besti_v[...] = jnp.where(better, (NB - 1) * TM + qd * QR + pos, besti_v[...])
        bv = best_v[...]
        mx = jnp.max(bv, axis=0, keepdims=True)
        idx = jnp.min(jnp.where(bv == mx, besti_v[...], S), axis=0, keepdims=True)[0, 0]
        idx = jnp.minimum(idx, S - 1)
        base = pl.multiple_of((idx // 16) * 16, 16)
        pb = pl.ds(pl.multiple_of(base // 2, 8), 8)
        x1 = _bf(x1_v[pb, :]).astype(f32)
        hsel = _bf(h2_v[pb, :])
        h2 = hsel.astype(f32)
        r_sel = mx[:, 0:1]
        for n in range(NFP):
            for d in cp_ffn(n):
                d.wait()
        acts, y = [], None
        for n in range(NFP + 1):
            if n < NFP:
                cols = slice(n * FP, (n + 1) * FP)
                gg = jnp.dot(hsel, _bf(wg_v[:, cols]), preferred_element_type=f32)
                uu = jnp.dot(hsel, _bf(wu_v[:, cols]), preferred_element_type=f32)
                acts.append((gg * jax.nn.sigmoid(gg) * uu).astype(bf16))
            if n > 0:
                part = jnp.dot(acts[n - 1], _bf(wd_v[(n - 1) * FP // 2:n * FP // 2, :]), preferred_element_type=f32)
                y = part if y is None else y + part
        y = y * jax.nn.sigmoid(r_sel)
        rows = base + lax.broadcasted_iota(i32, (16, D), 0)
        new = (x1 + gb * (h2 + y)).astype(bf16)
        for i in range(NB):
            cp_out(i).wait()
        out_v[pb, :] = pltpu.bitcast(jnp.where(rows == idx, new, _bf(out_v[pb, :])), u32)
        fin = pltpu.make_async_copy(out_v.at[pb, :].bitcast(bf16), out_hbm.at[pl.ds(base, 16), :], sems.at[S_FIN])
        fin.start()
        fin.wait()


@jax.jit
def pallas_adaLN_cond__sliding_block_cached__moe_arch_mod__prompt_kernel(
    A_x, A_k_cache, A_v_cache, A_wq, A_wo, B_x, B_w_r, B_w_gate, B_w_up, B_w_down, c, w_mod,
):
    anyspec = pl.BlockSpec(memory_space=pl.ANY)
    out = pl.pallas_call(
        _kernel,
        out_shape=jax.ShapeDtypeStruct((S, D), bf16),
        in_specs=[anyspec] * 11,
        out_specs=anyspec,
        scratch_shapes=[
            pltpu.VMEM((S // 2, D), u32),
            pltpu.VMEM((HKV, W // 2, DH), u32),
            pltpu.VMEM((HKV, W // 2, DH), u32),
            pltpu.VMEM((D // 2, HQ * DH), u32),
            pltpu.VMEM((HQ * DH // 2, D), u32),
            pltpu.VMEM((D,), bf16),
            pltpu.VMEM((D // 2, F), u32),
            pltpu.VMEM((D // 2, F), u32),
            pltpu.VMEM((F // 2, D), u32),
            pltpu.VMEM((1, D), bf16),
            pltpu.VMEM((D // 2, 6 * D), u32),
            pltpu.VMEM((TM // 2, D), u32),
            pltpu.VMEM((2, 7, HM // 2, HK), u32),
            pltpu.VMEM((5, HM // 2, HK), u32),
            pltpu.VMEM((2, HM // 2, HK), u32),
            pltpu.VMEM((TM // 2, GW), u32),
            pltpu.VMEM((TM, 2 * DH), f32),
            pltpu.VMEM((TM, HK), f32),
            pltpu.VMEM((HKV, 5, HK // 2, HK), u32),
            pltpu.VMEM((HKV, 5, HK // 2, HK), u32),
            pltpu.VMEM((2, TM, D), f32),
            pltpu.VMEM((S // 2 + TM // 2, D), u32),
            pltpu.VMEM((S // 2 + TM // 2, D), u32),
            pltpu.VMEM((S // 2 + TM // 2, D), u32),
            pltpu.VMEM((8, 6 * D), f32),
            pltpu.VMEM((QR, 128), f32),
            pltpu.VMEM((QR, 128), i32),
            pltpu.VMEM((8, 128), u32),
            pltpu.SMEM((8,), i32),
            pltpu.SemaphoreType.DMA((NSEM,)),
        ],
        compiler_params=pltpu.CompilerParams(vmem_limit_bytes=120 * 1024 * 1024),
    )(
        A_x.reshape(S, D), A_k_cache.reshape(HKV, SK, DH), A_v_cache.reshape(HKV, SK, DH),
        A_wq, A_wo, B_w_r, B_w_gate, B_w_up, B_w_down, c, w_mod,
    )
    return out.reshape(1, S, D)
```

```python
import jax
import jax.numpy as jnp
from jax import lax
import jax.experimental.pallas as pl
import jax.experimental.pallas.tpu as pltpu

S, D, HQ, HKV, DH, SK, W, F = 2048, 1024, 32, 4, 128, 2048, 512, 3584
REP = HQ // HKV
GW = REP * DH
TM = 512
NB = S // TM
QR = TM // HKV
HM = TM // 2
HK = D // 2
WPARTS = 8
SIDE_STRIDE = 7
SIDE_DIST = 4
CR = 32
SR = 16
NSL = HM // HKV // SR
LOG2E = 1.4426950408889634
QSCALE = (DH ** -0.5) * LOG2E
EPS = 1e-5
f32, bf16, u32, i32 = jnp.float32, jnp.bfloat16, jnp.uint32, jnp.int32

S_C, S_WMS, S_WMC, S_X0, S_X2, S_WR, S_FIN, S_WQ0 = range(8)
S_WQ = 8
S_WO = S_WQ + 2 * HKV
S_K = S_WO + HKV
S_V = S_K + HKV
S_X1 = S_V + HKV
S_WMB = S_X1 + 2 * HKV
S_OUT = S_WMB + HKV
S_WG, S_WU, S_WD = range(S_OUT + NB, S_OUT + NB + 3)
NSEM = S_WD + 1
NFP = 7
FP = F // NFP


def _ln(x):
    m = jnp.mean(x, axis=-1, keepdims=True)
    xc = x - m
    v = jnp.mean(xc * xc, axis=-1, keepdims=True)
    return xc * lax.rsqrt(v + EPS)


def _packs(y):
    r, c = y.shape
    y4 = y.reshape(r // 16, 2, 8, c)
    return pltpu.pack_elementwise([y4[:, 0].reshape(r // 2, c), y4[:, 1].reshape(r // 2, c)], packed_dtype=bf16)


def _halves(w):
    return tuple(pltpu.unpack_elementwise(w, index=n, packed_dtype=bf16, unpacked_dtype=f32) for n in range(2))


def _unpacks(w):
    r, c = w.shape
    lo, hi = (t.reshape(r // 8, 8, c) for t in _halves(w))
    return jnp.stack([lo, hi], axis=1).reshape(2 * r, c)


def _bf(x):
    return pltpu.bitcast(x, bf16)


def _mo(x, m):
    return x if isinstance(x, int) else pl.multiple_of(x, m)


def _recip(l):
    r = pl.reciprocal(l, approx=True)
    return r * (2.0 - l * r)


def _kernel(x_hbm, k_hbm, v_hbm, wq_hbm, wo_hbm, wr_hbm, wg_hbm, wu_hbm, wd_hbm, c_hbm, wm_hbm,
            out_hbm,
            x_v, k_v, v_v, wq_v, wo_v, wr_v, wg_v, wu_v, wd_v, c_v, wm_v,
            h_v, h7_v, o7_v, o7a_v, q_v, qp_v, ost_v, bq_v, bo_v, acc_v, out_v, x1_v, h2_v, mod_v, best_v, besti_v, zero_v, zs_ref, sems):
    def cp(src, dst, i):
        return pltpu.make_async_copy(src, dst.bitcast(bf16), sems.at[i])

    def cp_rows(hbm, vm, r0, n, i):
        return cp(hbm.at[pl.ds(_mo(r0, n), n), :], vm.at[pl.ds(_mo(r0 // 2, n // 2), n // 2), :], i)

    def cp_cols(hbm, vm, c0, n, i):
        return cp(hbm.at[:, pl.ds(_mo(c0, 128), n)], vm.at[:, pl.ds(_mo(c0, 128), n)], i)

    def cp_wq(g, half):
        return cp_cols(wq_hbm, wq_v, g * GW + half * (GW // 2), GW // 2, S_WQ + 2 * g + half)

    def cp_k(g):
        return cp(k_hbm.at[g, pl.ds(SK - W, W), :], k_v.at[g], S_K + g)

    def cp_v(g):
        return cp(v_hbm.at[g, pl.ds(SK - W, W), :], v_v.at[g], S_V + g)

    def cp_x1(g, half):
        n = HM // HKV
        return cp_rows(x_hbm, x_v, TM + half * HM + g * n, n, S_X1 + 2 * g + half)


    def cp_wo(g):
        return cp_rows(wo_hbm, wo_v, g * GW, GW, S_WO + g)

    def cp_out(i):
        r0 = i * TM
        return pltpu.make_async_copy(out_v.at[pl.ds(_mo(r0 // 2, TM // 2), TM // 2), :].bitcast(bf16),
                                     out_hbm.at[pl.ds(_mo(r0, TM), TM), :], sems.at[S_OUT + i])

    cp_c = pltpu.make_async_copy(c_hbm, c_v, sems.at[S_C])
    cp_wr = pltpu.make_async_copy(wr_hbm, wr_v, sems.at[S_WR])
    cp_wms = cp_cols(wm_hbm, wm_v, 0, D, S_WMS)
    cp_wmc = cp_cols(wm_hbm, wm_v, D, D, S_WMC)
    cp_x0 = cp_rows(x_hbm, x_v, 0, TM, S_X0)
    cp_x2 = cp_rows(x_hbm, x_v, 2 * TM, S - 2 * TM, S_X2)

    def cp_wmb(n):
        return cp_cols(wm_hbm, wm_v, (2 + n) * D, D, S_WMB + n)

    def cp_ffn():
        return (cp(wg_hbm, wg_v, S_WG), cp(wu_hbm, wu_v, S_WU), cp(wd_hbm, wd_v, S_WD))

    def group_set(g):
        return (cp_wq(g, 0), cp_x1(g, 0), cp_x1(g, 1), cp_wq(g, 1), cp_k(g), cp_v(g), cp_wo(g))


    cp_wq00 = cp_cols(wq_hbm, wq_v, 0, DH, S_WQ0)
    cp_wq01 = cp_cols(wq_hbm, wq_v, DH, GW // 2 - DH, S_WQ)
    for d in (cp_c, cp_wr, cp_x0, cp_wms, cp_wmc, cp_x1(0, 0), cp_x1(0, 1), cp_wq00, cp_wq01, cp_wq(0, 1),
              cp_k(0), cp_v(0), cp_wo(0)):
        d.start()
    for g in range(1, HKV):
        for d in group_set(g) + (cp_wmb(g - 1),):
            d.start()
    for d in (cp_x2, cp_wmb(HKV - 1)) + cp_ffn():
        d.start()
    best_v[...] = jnp.full(best_v.shape, -jnp.inf, f32)
    besti_v[...] = jnp.zeros(besti_v.shape, i32)
    zero_v[...] = jnp.zeros(zero_v.shape, u32)
    mod_v[...] = jnp.zeros(mod_v.shape, f32)
    q_v[0:8, 0:128] = jnp.zeros((8, 128), u32)
    qp_v[0:8, 0:128] = jnp.zeros((8, 128), f32)
    for n in range(8):
        zs_ref[n] = 0
    cp_c.wait()
    cp_wr.wait()
    cc = c_v[...].astype(f32)
    sc = jnp.broadcast_to((cc * jax.nn.sigmoid(cc)).astype(bf16), (16, D))
    cp_x0.wait()
    acc_v[1] = _ln(_bf(x_v[0:TM // 2, :]).astype(f32))
    cp_wms.wait()
    mod_v[:, 0:D] = jnp.dot(sc, _bf(wm_v[:, 0:D]), preferred_element_type=f32)[0:8]
    cp_wmc.wait()
    mod_v[:, D:2 * D] = jnp.dot(sc, _bf(wm_v[:, D:2 * D]), preferred_element_type=f32)[0:8]
    h_v[...] = _packs(acc_v[1] * (1.0 + mod_v[0:1, D:2 * D]) + mod_v[0:1, 0:D])

    def ln1_slice(row0, slot, dst0, normed=False, gate=None):
        sa = mod_v[0:1, 0 * D:1 * D]
        ca1 = 1.0 + mod_v[0:1, 1 * D:2 * D]
        if normed:
            xt, xb = acc_v[1, row0:row0 + 16, :], acc_v[1, row0 + HM:row0 + HM + 16, :]
            norm = lambda t: t
        else:
            xt, xb = (_bf(x_v[pl.ds(_mo(r // 2, 8), 8), :] | gate).astype(f32) for r in (row0, row0 + HM))
            norm = _ln
        dst = pl.ds(_mo(dst0 // 2, 8), 8)
        hs_ = []
        for r in (0, 8):
            top = norm(xt[r:r + 8]) * ca1 + sa
            bot = norm(xb[r:r + 8]) * ca1 + sa
            a11, a12, a21, a22 = top[:, :HK], top[:, HK:], bot[:, :HK], bot[:, HK:]
            hs_.append((a11 + a22, a21 + a22, a11, a22, a11 + a12, a21 - a11, a12 - a22))
        for n in range(7):
            h7_v[slot, n, dst, :] = pltpu.pack_elementwise([hs_[0][n], hs_[1][n]], packed_dtype=bf16)

    def wsum_slice(halves, dst):
        nr = dst.shape[1]
        for rr in range(0, nr, 8):
            for c in range(0, HK, 128):
                b11, b12, b21, b22 = (_halves(halves[kh][rr:rr + 8, nh * HK + c:nh * HK + c + 128])
                                      for kh in range(2) for nh in range(2))
                for n, (p, q, sign) in enumerate(((b11, b22, 1), (b12, b22, -1), (b21, b11, -1),
                                                  (b11, b12, 1), (b21, b22, 1))):
                    dst[n, rr:rr + 8, c:c + 128] = pltpu.pack_elementwise(
                        [u + w if sign > 0 else u - w for u, w in zip(p, q)], packed_dtype=bf16)

    def epi_rows16(src0, row0, slot, acc0, pos0, valid, gate):
        ga = mod_v[0:1, 2 * D:3 * D]
        sb = mod_v[0:1, 3 * D:4 * D]
        cb1 = 1.0 + mod_v[0:1, 4 * D:5 * D]
        gb = mod_v[0:1, 5 * D:6 * D]
        wr = wr_v[...].astype(f32).reshape(1, D)
        rows = pl.ds(_mo(row0 // 2, 8), 8)
        xw = x_v[pl.ds(_mo(src0 // 2, 8), 8), :]
        xs = _halves(xw if isinstance(gate, int) else xw | gate)
        x1s, outs, h2s = [], [], []
        for n in range(2):
            x1 = xs[n] + ga * acc_v[slot, pl.ds(_mo(acc0 + 8 * n, 8), 8), :]
            h2 = _ln(x1) * cb1 + sb
            x1s.append(x1)
            h2s.append(h2)
            outs.append(x1 + gb * h2)
            r = jnp.broadcast_to(jnp.sum(h2 * wr, axis=-1, keepdims=True), (8, 128))
            ib = row0 + n + 2 * lax.broadcasted_iota(i32, (8, 128), 0)
            sl = pl.ds(pos0 + 8 * n, 8)
            better = r > best_v[sl, :]
            if valid is not True:
                better = better & valid
            best_v[sl, :] = jnp.where(better, r, best_v[sl, :])
            besti_v[sl, :] = jnp.where(better, ib, besti_v[sl, :])
        x1_v[rows, :] = pltpu.pack_elementwise(x1s, packed_dtype=bf16)
        out_v[rows, :] = pltpu.pack_elementwise(outs, packed_dtype=bf16)
        h2_v[rows, :] = pltpu.pack_elementwise(h2s, packed_dtype=bf16)

    def wq_quad(g):
        def quad(kh, nh, r0=0, nr=HK // 2, c=0, nc=HK):
            return wq_v[pl.ds(_mo(kh * (HK // 2) + r0, 8), nr), pl.ds(_mo(g * GW + nh * HK + c, DH), nc)]
        return quad

    def wo_quad(g):
        def quad(kh, nh, r0=0, nr=HK // 2, c=0, nc=HK):
            return wo_v[pl.ds(_mo((g * GW + kh * HK) // 2 + r0, 8), nr), pl.ds(_mo(nh * HK + c, DH), nc)]
        return quad

    def b_operand(quad, sums, g, n, j):
        if n == 1:
            return quad(0, 0, c=j * DH, nc=DH)
        if n == 4:
            return quad(1, 1, c=j * DH, nc=DH)
        return sums[g, (0, None, 1, 2, None, 3, 4)[n], :, j * DH:(j + 1) * DH]

    def prep_part(g, part, do_q=True, do_o=True):
        nr = HK // 2 // WPARTS
        r0 = part * nr
        rows = pl.ds(_mo(r0, nr), nr)
        if do_q:
            wsum_slice([wq_v.at[pl.ds(_mo(kh * (HK // 2) + r0, nr), nr), pl.ds(_mo(g * GW, GW), GW)]
                        for kh in range(2)], bq_v.at[g, :, rows, :])
        if do_o:
            wsum_slice([wo_v.at[pl.ds(_mo((g * GW + kh * HK) // 2 + r0, nr), nr), :]
                        for kh in range(2)], bo_v.at[g, :, rows, :])

    def period(i, g, mode):
        hs = i % 2
        if mode == 2:
            @pl.when(i == 0)
            def _():
                for d in group_set(g):
                    d.wait()
                cp_wmb(g - 1).wait()
                for part in range(WPARTS):
                    mc = pl.ds(pl.multiple_of((1 + g) * D + part * (D // WPARTS), DH), D // WPARTS)
                    mod_v[:, mc] = jnp.dot(sc, _bf(wm_v[:, mc]), preferred_element_type=f32)[0:8]
                    prep_part(g, part)

            @pl.when((i == 1) & (g == 0))
            def _():
                cp_wmb(HKV - 1).wait()
                cp_x2.wait()
                for part in range(WPARTS):
                    mc = slice(5 * D + part * (D // WPARTS), 5 * D + (part + 1) * (D // WPARTS))
                    mod_v[:, mc] = jnp.dot(sc, _bf(wm_v[:, mc]), preferred_element_type=f32)[0:8]
                    prep_part(0, part, do_o=False)

            @pl.when((g == 0) & (i >= 2))
            def _():
                cp_out(i - 2).start()

        zero = zero_v[...]
        zz = [zs_ref[n] for n in range(8)]
        zs = zz[0]

        def ln_work(sub, dz):
            q0 = g * (HM // HKV) + sub * SR
            ln1_slice(jnp.minimum(i + 1, NB - 1) * TM + q0, 1 - hs, q0, gate=dz)
            return h7_v[1 - hs, 0, pl.ds(pl.multiple_of(q0 // 2 + zs, 8), 8), 0:128]

        def epi_work(sub, dz):
            toks = None
            for half in range(2):
                q0 = half * HM + g * (HM // HKV) + sub * SR
                src0 = jnp.maximum(i - 1, 0) * TM + q0
                row0 = jnp.where(i == 0, S, (i - 1) * TM) + q0
                pos = (2 * sub + half) * SR
                epi_rows16(src0, row0, 1 - hs, q0, pos, i > 0, dz)
                opq = pl.ds(pl.multiple_of(row0 // 2 + zs, 8), 8)
                ob = pl.ds(pl.multiple_of(pos + zs, 8), 8)
                t = (out_v[opq, 0:128] | x1_v[opq, 0:128]
                     | pltpu.bitcast(best_v[ob, :], u32) | pltpu.bitcast(besti_v[ob, :], u32))
                toks = t if toks is None else toks | t
            return toks

        early, late = [], []
        if mode == 2:
            for sub in range(NSL):
                early += [lambda dz, sub=sub: epi_work(sub, dz)] + [None] * (SIDE_STRIDE - 1)
                late += [lambda dz, sub=sub: ln_work(sub, dz)] + [None] * (SIDE_STRIDE - 1)
        else:
            def h7_first(n):
                ln1_slice(n * SR, 0, n * SR, normed=True)
                return h7_v[0, 0, pl.ds(pl.multiple_of(n * (SR // 2) + zs, 8), 8), 0:128]
            for sub in range(NSL):
                early.append(lambda dz, sub=sub: ln_work(sub, dz))
            for n in range(HM // SR):
                early.append(lambda dz, n=n: h7_first(n))
        pending = [None] * (SIDE_DIST if mode == 2 else 2)

        def anchored(w, extra=None):
            tok = pending.pop(0) if pending else None
            if extra is not None:
                tok = extra if tok is None else tok | extra
            if tok is not None:
                w = jnp.concatenate([w[0:8, :] | jnp.tile(tok & zero, (1, w.shape[1] // 128)), w[8:, :]], axis=0)
            return _bf(w)

        def after(res, queue):
            work = queue.pop(0) if queue else None
            if work is not None:
                src = (qp_v.at[:, 0:128] if queue is early else acc_v.at[hs, :, 0:128]) if mode == 2 else q_v.at[:, 0:128]
                gate = pltpu.bitcast(src[pl.ds(pl.multiple_of(zs, 8), 8), :], u32) & zero
                pending.append(work(jnp.tile(gate, (1, D // 128))))
            else:
                pending.append(None)

        def mm(a, w, queue, extra=None):
            res = jnp.dot(a, anchored(w, extra), preferred_element_type=f32)
            after(res, queue)
            return res

        if mode == 0:
            for hh in range(REP):
                if hh == 0:
                    waits = (cp_x1(0, 0), cp_x1(0, 1), cp_wq00)
                elif hh == 1:
                    waits = (cp_wq01,)
                elif hh == REP // 2:
                    waits = (cp_wq(0, 1), cp_k(0), cp_v(0))
                else:
                    waits = ()
                for d in waits:
                    d.wait()
                h = _bf(h_v[pl.ds(pl.multiple_of(zz[hh], 8), TM // 2), :])
                qh = mm(h, wq_v[:, pl.ds(_mo(g * GW + hh * DH, DH), DH)], early)
                q_v[:, hh * DH:(hh + 1) * DH] = _packs(qh * QSCALE)
        else:
            quad = wq_quad(g)
            for j in range(HK // DH):
                def d(n):
                    return mm(_bf(h7_v[hs + zz[j], n]), b_operand(quad, bq_v, g, n, j), early)
                L, R = pl.ds(0, DH), pl.ds(DH, DH)
                QL, QR_ = pl.ds(j * DH, DH), pl.ds(HK + j * DH, DH)
                def comb(m, *ops):
                    for r in range(0, HM, CR):
                        mc = m[r:r + CR]
                        for (row, col, kind, qsrc) in ops:
                            rows = pl.ds(row + r, CR)
                            if kind == "set":
                                qp_v[rows, col] = mc
                            elif kind == "add":
                                qp_v[rows, col] += mc
                            elif kind == "sub":
                                qp_v[rows, col] -= mc
                            else:
                                q_v[pl.ds((row + r) // 2, CR // 2), qsrc] = _packs((qp_v[rows, col] + mc) * QSCALE)
                comb(d(0), (0, L, "set", None), (HM, R, "set", None))
                comb(d(1), (HM, R, "sub", None), (HM, L, "set", None))
                comb(d(2), (HM, R, "add", None), (0, R, "set", None))
                comb(d(3), (0, L, "add", None), (HM, L, "q", QL))
                comb(d(4), (0, L, "sub", None), (0, R, "q", QR_))
                comb(d(5), (HM, R, "q", QR_))
                comb(d(6), (0, L, "q", QL))

        otok = None
        for hh in range(REP):
            s = lax.dot_general(_bf(q_v[:, hh * DH:(hh + 1) * DH]), anchored(k_v[g]), (((1,), (1,)), ((), ())), preferred_element_type=f32)
            after(s, early)
            m = jnp.max(s, axis=-1, keepdims=True)
            p = jnp.exp2(s - m)
            l = jnp.sum(p, axis=-1, keepdims=True)
            o = mm(p.astype(bf16), v_v[g], early, otok) * _recip(l)
            col = slice((hh % 4) * DH, (hh % 4 + 1) * DH)
            if hh < 4:
                top, bot = o[:HM], o[HM:]
                ost_v[:, col] = o
                o7a_v[0, :, col] = _packs(top)
                o7a_v[1, :, col] = _packs(bot - top)
                oref = o7a_v.at[1]
            else:
                a12, a22 = o[:HM], o[HM:]
                a11, a21 = ost_v[0:HM, col], ost_v[HM:TM, col]
                o7_v[0, :, col] = _packs(a11 + a22)
                o7_v[1, :, col] = _packs(a21 + a22)
                o7_v[2, :, col] = _packs(a22)
                o7_v[3, :, col] = _packs(a11 + a12)
                o7_v[4, :, col] = _packs(a12 - a22)
                oref = o7_v.at[4]
            otok = None
            if hh + 2 < REP:
                cc = (hh % 4) * DH
                otok = oref[pl.ds(pl.multiple_of(zs, 8), 8), pl.ds(pl.multiple_of(cc + zs * 128, DH), DH)]

        if mode == 0:
            cp_wo(0).wait()
            lax.fori_loop(0, WPARTS, lambda part, _: prep_part(0, part, do_q=False), None)
        quad = wo_quad(g)

        def d(n, j):
            if n in (2, 5):
                lhs = o7a_v[(0 if n == 2 else 1) + zz[j]]
            else:
                lhs = o7_v[(0, 1, None, 2, 3, None, 4)[n] + zz[j]]
            return mm(_bf(lhs), b_operand(quad, bo_v, g, n, j), late)

        def comb(m, j, *ops):
            for r in range(0, HM, CR):
                mc = m[r:r + CR]
                for (row, right, kind) in ops:
                    rows, col = pl.ds(row + r, CR), pl.ds(right * HK + j * DH, DH)
                    if kind == "first" and mode == 0:
                        acc_v[hs, rows, col] = mc
                    elif kind == "first":
                        acc_v[hs, rows, col] = jnp.where(g == 0, mc, acc_v[hs, rows, col] + mc)
                    elif kind == "add":
                        acc_v[hs, rows, col] += mc
                    else:
                        acc_v[hs, rows, col] -= mc
        for j in range(HK // DH):
            comb(d(2, j), j, (HM, 1, "first"), (0, 1, "first"))
            comb(d(5, j), j, (HM, 1, "add"))
        for j in range(HK // DH):
            comb(d(0, j), j, (0, 0, "first"), (HM, 1, "add"))
            comb(d(1, j), j, (HM, 1, "sub"), (HM, 0, "first"))
            comb(d(3, j), j, (0, 0, "add"), (HM, 0, "add"))
            comb(d(4, j), j, (0, 0, "sub"), (0, 1, "add"))
            comb(d(6, j), j, (0, 0, "add"))
        assert not any(early) and not any(late)

    with jax.named_scope("p00"):
        period(0, 0, 0)
    with jax.named_scope("loopB"):
        def step_b(t, _):
            period(t // HKV, t % HKV, 2)
        lax.fori_loop(1, NB * HKV, step_b, None)
    cp_out(NB - 2).start()

    with jax.named_scope("tail"):
        ga, sb, cb, gb = (mod_v[0:1, n * D:(n + 1) * D] for n in range(2, 6))
        wr = wr_v[...].astype(f32).reshape(1, D)
        last = pl.ds((NB - 1) * TM // 2, TM // 2)
        x1 = _unpacks(x_v[last, :]) + ga * acc_v[(NB - 1) % 2]
        x1_v[last, :] = _packs(x1)
        h2 = _ln(x1) * (1.0 + cb) + sb
        out_v[last, :] = _packs(x1 + gb * h2)
        h2_v[last, :] = _packs(h2)
        cp_out(NB - 1).start()
        r = jnp.broadcast_to(jnp.sum(h2 * wr, axis=-1, keepdims=True), (TM, 128))
        pos = lax.broadcasted_iota(i32, (QR, 128), 0)
        pos = (pos & ~15) + 2 * (pos & 7) + ((pos & 15) >> 3)
        for qd in range(HKV):
            rb = r[qd * QR:(qd + 1) * QR]
            better = rb > best_v[...]
            best_v[...] = jnp.where(better, rb, best_v[...])
            besti_v[...] = jnp.where(better, (NB - 1) * TM + qd * QR + pos, besti_v[...])
        bv = best_v[...]
        mx = jnp.max(bv, axis=0, keepdims=True)
        idx = jnp.min(jnp.where(bv == mx, besti_v[...], S), axis=0, keepdims=True)[0, 0]
        idx = jnp.minimum(idx, S - 1)
        base = pl.multiple_of((idx // 16) * 16, 16)
        pb = pl.ds(pl.multiple_of(base // 2, 8), 8)
        x1 = _bf(x1_v[pb, :]).astype(f32)
        hsel = _bf(h2_v[pb, :])
        h2 = hsel.astype(f32)
        r_sel = mx[:, 0:1]
        for d in cp_ffn():
            d.wait()
        acts, y = [], None
        for n in range(NFP + 1):
            if n < NFP:
                cols = slice(n * FP, (n + 1) * FP)
                gg = jnp.dot(hsel, _bf(wg_v[:, cols]), preferred_element_type=f32)
                uu = jnp.dot(hsel, _bf(wu_v[:, cols]), preferred_element_type=f32)
                acts.append((gg * jax.nn.sigmoid(gg) * uu).astype(bf16))
            if n > 0:
                part = jnp.dot(acts[n - 1], _bf(wd_v[(n - 1) * FP // 2:n * FP // 2, :]), preferred_element_type=f32)
                y = part if y is None else y + part
        y = y * jax.nn.sigmoid(r_sel)
        rows = base + lax.broadcasted_iota(i32, (16, D), 0)
        new = (x1 + gb * (h2 + y)).astype(bf16)
        for i in range(NB):
            cp_out(i).wait()
        out_v[pb, :] = pltpu.bitcast(jnp.where(rows == idx, new, _bf(out_v[pb, :])), u32)
        fin = pltpu.make_async_copy(out_v.at[pb, :].bitcast(bf16), out_hbm.at[pl.ds(base, 16), :], sems.at[S_FIN])
        fin.start()
        fin.wait()


@jax.jit
def pallas_adaLN_cond__sliding_block_cached__moe_arch_mod__prompt_kernel(
    A_x, A_k_cache, A_v_cache, A_wq, A_wo, B_x, B_w_r, B_w_gate, B_w_up, B_w_down, c, w_mod,
):
    anyspec = pl.BlockSpec(memory_space=pl.ANY)
    out = pl.pallas_call(
        _kernel,
        out_shape=jax.ShapeDtypeStruct((S, D), bf16),
        in_specs=[anyspec] * 11,
        out_specs=anyspec,
        scratch_shapes=[
            pltpu.VMEM((S // 2, D), u32),
            pltpu.VMEM((HKV, W // 2, DH), u32),
            pltpu.VMEM((HKV, W // 2, DH), u32),
            pltpu.VMEM((D // 2, HQ * DH), u32),
            pltpu.VMEM((HQ * DH // 2, D), u32),
            pltpu.VMEM((D,), bf16),
            pltpu.VMEM((D // 2, F), u32),
            pltpu.VMEM((D // 2, F), u32),
            pltpu.VMEM((F // 2, D), u32),
            pltpu.VMEM((1, D), bf16),
            pltpu.VMEM((D // 2, 6 * D), u32),
            pltpu.VMEM((TM // 2, D), u32),
            pltpu.VMEM((2, 7, HM // 2, HK), u32),
            pltpu.VMEM((5, HM // 2, HK), u32),
            pltpu.VMEM((2, HM // 2, HK), u32),
            pltpu.VMEM((TM // 2, GW), u32),
            pltpu.VMEM((TM, 2 * DH), f32),
            pltpu.VMEM((TM, HK), f32),
            pltpu.VMEM((HKV, 5, HK // 2, HK), u32),
            pltpu.VMEM((HKV, 5, HK // 2, HK), u32),
            pltpu.VMEM((2, TM, D), f32),
            pltpu.VMEM((S // 2 + TM // 2, D), u32),
            pltpu.VMEM((S // 2 + TM // 2, D), u32),
            pltpu.VMEM((S // 2 + TM // 2, D), u32),
            pltpu.VMEM((8, 6 * D), f32),
            pltpu.VMEM((QR, 128), f32),
            pltpu.VMEM((QR, 128), i32),
            pltpu.VMEM((8, 128), u32),
            pltpu.SMEM((8,), i32),
            pltpu.SemaphoreType.DMA((NSEM,)),
        ],
        compiler_params=pltpu.CompilerParams(vmem_limit_bytes=120 * 1024 * 1024),
    )(
        A_x.reshape(S, D), A_k_cache.reshape(HKV, SK, DH), A_v_cache.reshape(HKV, SK, DH),
        A_wq, A_wo, B_w_r, B_w_gate, B_w_up, B_w_down, c, w_mod,
    )
    return out.reshape(1, S, D)
```
